```python
import os as _os
_os.environ.setdefault("JAX_PLATFORMS", "cpu")
import jax
import jax.numpy as jnp

def _softmax(x, axis=-1):
    return jax.nn.softmax(x, axis=axis)
def _gelu(x):
    return jax.nn.gelu(x, approximate=True)
def _silu(x):
    return jax.nn.silu(x)
def _sigmoid(x):
    return jax.nn.sigmoid(x)
def _layernorm(x, axis=-1, eps=1e-5):
    m = jnp.mean(x, axis=axis, keepdims=True)
    v = jnp.var(x, axis=axis, keepdims=True)
    return (x - m) / jnp.sqrt(v + eps)
def _scatter_add(tgt, idx, src, axis=0):
    return tgt.at[idx].add(src)
def _segment_sum(src, seg, n):
    return jax.ops.segment_sum(src, seg, n)
class _Rng:
    def __init__(self, key):
        self._k = key
    def _next(self):
        self._k, sub = jax.random.split(self._k)
        return sub
    def normal(self, shape):
        return jax.random.normal(self._next(), shape, dtype=jnp.bfloat16)
    def randint(self, lo, hi, shape):
        return jax.random.randint(self._next(), shape, lo, hi, dtype=jnp.int32)
    def uniform(self, shape, lo=0.0, hi=1.0):
        return jax.random.uniform(self._next(), shape, jnp.bfloat16, lo, hi)
    def permutation(self, n):
        return jax.random.permutation(self._next(), n)


kernel_name = 'interleave_layers__sliding_local_dilated__mixer_channel_mlp__prompt'

def setup_inputs():
    _rng = _Rng(jax.random.key(int.from_bytes(__import__("os").urandom(4), "little")))
    _w = (lambda a: (lambda t: t.astype(jnp.bfloat16) if jnp.issubdtype(t.dtype, jnp.floating) else t)(jnp.asarray(a)))
    def _A_setup():
        B, S, D = 1, 2048, 512
        return {
            "x": _w((lambda *s: _rng.normal(s) * 0.05)(B, S, D)),
            "wqkv": _w((lambda *s: _rng.normal(s) * 0.05)(D, 3 * D)),
            "wo": _w((lambda *s: _rng.normal(s) * 0.05)(D, D)),
        }
    _A_in = _A_setup()

    def _B_setup():
        B, S, D, F = 1, 2048, 512, 1376
        return {
            "x": _w((lambda *s: _rng.normal(s) * 0.05)(B, S, D)),
            "w1": _w((lambda *s: _rng.normal(s) * 0.4)(D, F) * (D ** -0.5)),
            "b1": _w((lambda *s: _rng.normal(s) * 0.4)(F)),
            "w2": _w((lambda *s: _rng.normal(s) * 0.4)(F, D) * (F ** -0.5)),
            "b2": _w((lambda *s: _rng.normal(s) * 0.4)(D)),
        }
    _B_in = _B_setup()

    return {
        "A_x": _A_in["x"],
        "A_wqkv": _A_in["wqkv"],
        "A_wo": _A_in["wo"],
        "B_x": _B_in["x"],
        "B_w1": _B_in["w1"],
        "B_b1": _B_in["b1"],
        "B_w2": _B_in["w2"],
        "B_b2": _B_in["b2"],
    }

def reference(A_x, A_wqkv, A_wo, B_x, B_w1, B_b1, B_w2, B_b2):
    def _A_ref(x, wqkv, wo):
        B, S, D = x.shape
        H = 32; Dh = D // H
        W, dil = 8, 2
        qkv = (lambda x, *d: x.transpose(*d))((x @ wqkv).reshape(B, S, 3, H, Dh), 2, 0, 3, 1, 4)
        q, k, v = qkv[0], qkv[1], qkv[2]
        scale = Dh ** -0.5
        pos = jnp.arange(S)
        off = jnp.arange(W) * dil
        idx = pos[:, None] - off[None, :]
        mask = idx >= 0
        idx_c = jnp.where(mask, idx, 0).reshape(-1)
        kg = k[:, :, idx_c, :].reshape(B, H, S, W, Dh)
        vg = v[:, :, idx_c, :].reshape(B, H, S, W, Dh)
        logits = jnp.einsum("bhsd,bhswd->bhsw", q, kg) * scale
        logits = jnp.where(mask[None, None, :, :], logits, -1e9)
        attn = _softmax(logits, axis=-1)
        o = jnp.einsum("bhsw,bhswd->bhsd", attn, vg)
        return (lambda x, *d: x.transpose(*d))(o, 0, 2, 1, 3).reshape(B, S, D) @ wo

    def _B_ref(x, w1, b1, w2, b2):
        y = _layernorm(x, axis=-1)
        h = _gelu(jnp.einsum("bsd,df->bsf", y, w1) + b1)
        return jnp.einsum("bsf,fd->bsd", h, w2) + b2

    x = A_x
    x = x + _A_ref(_layernorm(x, axis=-1), A_wqkv, A_wo)
    x = x + _B_ref(_layernorm(x, axis=-1), B_w1, B_b1, B_w2, B_b2)
    x = x + _A_ref(_layernorm(x, axis=-1), A_wqkv, A_wo)
    x = x + _B_ref(_layernorm(x, axis=-1), B_w1, B_b1, B_w2, B_b2)
    return x
```

```python
import functools
import math

import jax
import jax.numpy as jnp
import jax.experimental.pallas as pl
import jax.experimental.pallas.tpu as pltpu

H = 32
W = 8
DIL = 2
HALO = 16
EPS = 1e-5
LANES = 128


def _layernorm(x):
    m = jnp.mean(x, axis=-1, keepdims=True)
    xc = x - m
    v = jnp.mean(xc * xc, axis=-1, keepdims=True)
    return xc * jax.lax.rsqrt(v + EPS)


def _gelu(x):
    c = math.sqrt(2.0 / math.pi)
    inner = x * (c + (c * 0.044715) * (x * x))
    hx = 0.5 * x
    return hx + hx * jnp.tanh(inner)


def _kernel(x_ref, wqkv_ref, wo_ref, w1_ref, b1_ref, w2_ref, b2_ref, o_ref,
            kv0_ref, kv1_ref, q_ref, att_ref, *, T, D, CH):
    step = pl.program_id(0)
    NT = D // LANES
    Dh = D // H
    qscale = (Dh ** -0.5) * math.log2(math.e)

    @pl.when(step == 0)
    def _():
        kv0_ref[:, 0:HALO, :] = jnp.zeros((2 * NT, HALO, LANES), jnp.float32)
        kv1_ref[:, 0:HALO, :] = jnp.zeros((2 * NT, HALO, LANES), jnp.float32)

    def attention(x, kv_ref):
        xn = _layernorm(x).astype(jnp.bfloat16)
        qkv = jnp.dot(xn, wqkv_ref[...], preferred_element_type=jnp.float32)
        for t in range(NT):
            q_ref[t] = qkv[:, t * LANES:(t + 1) * LANES] * qscale
        for t in range(2 * NT):
            kv_ref[t, HALO:HALO + T, :] = qkv[:, D + t * LANES:D + (t + 1) * LANES]
        for c in range(T // CH):
            r0 = c * CH
            q = [q_ref[t, r0:r0 + CH, :] for t in range(NT)]
            logits = []
            for w in range(W):
                s0 = HALO + r0 - DIL * w
                acc = q[0] * kv_ref[0, s0:s0 + CH, :]
                for t in range(1, NT):
                    acc = acc + q[t] * kv_ref[t, s0:s0 + CH, :]
                acc = acc + pltpu.roll(acc, 64, 1)
                acc = acc + pltpu.roll(acc, 32, 1)
                if r0 < DIL * w:
                    row = step * T + r0 + jax.lax.broadcasted_iota(jnp.int32, (CH, LANES), 0)
                    acc = jnp.where(row >= DIL * w, acc, -1e9 * math.log2(math.e))
                logits.append(acc)
            m = logits[0]
            for w in range(1, W):
                m = jnp.maximum(m, logits[w])
            p = [jnp.exp2(l - m) for l in logits]
            den = p[0]
            for w in range(1, W):
                den = den + p[w]
            inv = 1.0 / den
            for t in range(NT):
                s0 = HALO + r0
                acc = p[0] * kv_ref[NT + t, s0:s0 + CH, :]
                for w in range(1, W):
                    s0 = HALO + r0 - DIL * w
                    acc = acc + p[w] * kv_ref[NT + t, s0:s0 + CH, :]
                att_ref[r0:r0 + CH, t * LANES:(t + 1) * LANES] = (acc * inv).astype(jnp.bfloat16)
        kv_ref[:, 0:HALO, :] = kv_ref[:, T:T + HALO, :]
        return jnp.dot(att_ref[...], wo_ref[...], preferred_element_type=jnp.float32)

    def mlp(x):
        y = _layernorm(_layernorm(x)).astype(jnp.bfloat16)
        h = jnp.dot(y, w1_ref[...], preferred_element_type=jnp.float32)
        h = _gelu(h + b1_ref[...].astype(jnp.float32)).astype(jnp.bfloat16)
        o = jnp.dot(h, w2_ref[...], preferred_element_type=jnp.float32)
        return o + b2_ref[...].astype(jnp.float32)

    x = x_ref[...].astype(jnp.float32)
    x = x + attention(x, kv0_ref)
    x = x + mlp(x)
    x = x + attention(x, kv1_ref)
    x = x + mlp(x)
    o_ref[...] = x.astype(o_ref.dtype)


@jax.jit
def pallas_interleave_layers__sliding_local_dilated__mixer_channel_mlp__prompt_kernel(
    A_x: jax.Array,
    A_wqkv: jax.Array,
    A_wo: jax.Array,
    B_x: jax.Array,
    B_w1: jax.Array,
    B_b1: jax.Array,
    B_w2: jax.Array,
    B_b2: jax.Array,
):
    B, S, D = A_x.shape
    F = B_w1.shape[1]
    Dh = D // H
    assert B == 1
    T = 256
    CH = 16
    NT = D // LANES

    wqkv = A_wqkv.reshape(D, 3, H, Dh).transpose(0, 1, 3, 2).reshape(D, 3 * D)
    wo = A_wo.reshape(H, Dh, D).transpose(1, 0, 2).reshape(D, D)

    full = lambda shape: pl.BlockSpec(shape, lambda i: (0,) * len(shape))
    out = pl.pallas_call(
        functools.partial(_kernel, T=T, D=D, CH=CH),
        grid=(S // T,),
        in_specs=[
            pl.BlockSpec((T, D), lambda i: (i, 0)),
            full((D, 3 * D)),
            full((D, D)),
            full((D, F)),
            full((1, F)),
            full((F, D)),
            full((1, D)),
        ],
        out_specs=pl.BlockSpec((T, D), lambda i: (i, 0)),
        out_shape=jax.ShapeDtypeStruct((S, D), A_x.dtype),
        scratch_shapes=[
            pltpu.VMEM((2 * NT, T + HALO, LANES), jnp.float32),
            pltpu.VMEM((2 * NT, T + HALO, LANES), jnp.float32),
            pltpu.VMEM((NT, T, LANES), jnp.float32),
            pltpu.VMEM((T, D), jnp.bfloat16),
        ],
        compiler_params=pltpu.CompilerParams(
            dimension_semantics=("arbitrary",),
            vmem_limit_bytes=100 * 1024 * 1024,
        ),
    )(A_x.reshape(S, D), wqkv, wo, B_w1, B_b1.reshape(1, F), B_w2, B_b2.reshape(1, D))
    return out.reshape(B, S, D)
```

```python
import functools
import math

import jax
import jax.numpy as jnp
import jax.experimental.pallas as pl
import jax.experimental.pallas.tpu as pltpu

H = 32
W = 8
DIL = 2
HALO = 16
EPS = 1e-5
LANES = 128
TS = 256
WO_PITCH = 17
LOG2E = math.log2(math.e)


def _layernorm(x):
    m = jnp.mean(x, axis=-1, keepdims=True)
    xc = x - m
    v = jnp.mean(xc * xc, axis=-1, keepdims=True)
    return xc * jax.lax.rsqrt(v + EPS)


def _gelu_x2(x):
    c = math.sqrt(2.0 / math.pi)
    inner = x * (c + (c * 0.044715) * (x * x))
    return x + x * jnp.tanh(inner)


def _cat(ref, lo, n):
    return jnp.concatenate([ref[lo + t] for t in range(n)], axis=1)


def _kernel(x_hbm, wqkv_hbm, wo_hbm, w1_hbm, b1_hbm, w2_hbm, b2_hbm, o_hbm,
            kv0_ref, kv1_ref, q0_ref, q1_ref, att0_ref, att1_ref,
            xa_ref, xb_ref, xn_ref, wqkv_ref, wo_ref, tmp_ref,
            x_ref, o_ref, wqkv_in, wo_in, w1_ref, w2_ref, b1_ref, b2_ref,
            never_ref, isem, osem, *, D, NBLK):
    NT = D // LANES
    Dh = D // H
    qscale = (Dh ** -0.5) * LOG2E
    f32 = jnp.float32
    bf16 = jnp.bfloat16

    def slab_copies(src, col0, dst, slab0, sem0):
        return [pltpu.make_async_copy(src.at[:, pl.ds(col0 + t * LANES, LANES)],
                                      dst.at[slab0 + t], isem.at[sem0 + t])
                for t in range(NT)]

    wq_cp, wk_cp, wv_cp = [slab_copies(wqkv_hbm, j * D, wqkv_in, j * NT, j * NT)
                           for j in range(3)]
    w1_cp = slab_copies(w1_hbm, 0, w1_ref, 0, 3 * NT)
    w2_cp = slab_copies(w2_hbm, 0, w2_ref, 0, 4 * NT)
    wo_cp = [pltpu.make_async_copy(wo_hbm, wo_in, isem.at[5 * NT])]
    b_cp = [pltpu.make_async_copy(b1_hbm, b1_ref, isem.at[5 * NT + 1]),
            pltpu.make_async_copy(b2_hbm, b2_ref, isem.at[5 * NT + 2])]
    x_cp = [pltpu.make_async_copy(x_hbm.at[pl.ds(i * TS, TS), :], x_ref.at[i],
                                  isem.at[5 * NT + 3 + i]) for i in range(NBLK)]

    def o_copy(i):
        return pltpu.make_async_copy(o_ref.at[i], o_hbm.at[pl.ds(i * TS, TS), :], osem.at[i])

    o_last = [pltpu.make_async_copy(
        o_ref.at[NBLK - 1, :, pl.ds(t * LANES, LANES)],
        o_hbm.at[pl.ds((NBLK - 1) * TS, TS), pl.ds(t * LANES, LANES)],
        osem.at[NBLK - 1 + t]) for t in range(NT)]

    def start(cps):
        for c in cps:
            c.start()

    def wait(cps):
        for c in cps:
            c.wait()

    kvs = (kv0_ref, kv1_ref)
    qs = (q0_ref, q1_ref)
    atts = (att0_ref, att1_ref)

    def permute_cols(j):
        lane = jax.lax.broadcasted_iota(jnp.int32, (1, LANES), 1)
        pgrp = (lane % 16) // 4
        a = []
        for i in range(NT):
            ai = pltpu.bitcast(wqkv_in[j * NT + i], jnp.uint32)
            a.append(pltpu.roll(ai, 4 * i, 1) if i else ai)
        for t in range(NT):
            c = a[(0 - t) % 4]
            for p in range(1, 4):
                c = jnp.where(pgrp == p, a[(p - t) % 4], c)
            l2 = jax.lax.broadcasted_iota(jnp.int32, c.shape, 1)
            hh = l2 % H
            src = ((hh % 8) * 16 + 4 * t + l2 // H + 4 * (hh // 8)) & (LANES - 1)
            wqkv_ref[j * NT + t] = pltpu.bitcast(jnp.take_along_axis(c, src, axis=1), bf16)

    def permute_rows():
        for t in range(NT):
            for h in range(H):
                tmp_ref[t, h * WO_PITCH:h * WO_PITCH + Dh, :] = (
                    wo_in[h * Dh:(h + 1) * Dh, t * LANES:(t + 1) * LANES].astype(f32))
        for d in range(Dh):
            for t in range(NT):
                wo_ref[t, d * H:(d + 1) * H, :] = (
                    tmp_ref[t, pl.ds(d, H, stride=WO_PITCH), :].astype(bf16))

    def proj(xn, j, l, base, t0=0, nt=NT):
        r = jnp.dot(xn, _cat(wqkv_ref, j * NT + t0, nt), preferred_element_type=f32)
        for t in range(t0, t0 + nt):
            rt = r[:, (t - t0) * LANES:(t - t0 + 1) * LANES]
            if j == 0:
                qs[l][t, base:base + TS, :] = rt
            else:
                kvs[l][(j - 1) * NT + t, HALO + base:HALO + base + TS, :] = rt

    def qkv(xn, l):
        proj(xn, 1, l, 0)
        proj(xn, 0, l, 0)
        proj(xn, 2, l, 0)

    def att(l, base, first, CH=8, NB=3):
        kv_ref = kvs[l]
        never = jnp.broadcast_to(never_ref[...], (CH, LANES)) > 0
        dens = {}
        pend = {}
        for c in range(TS // CH):
            o0 = c * CH
            r0 = base + o0
            sc = jnp.where(never, dens[c - NB], qscale) if (NB and c >= NB) else qscale
            q = [qs[l][t, r0:r0 + CH, :] * sc for t in range(NT)]
            logits = []
            for w in range(W):
                s0 = HALO + r0 - DIL * w
                acc = q[0] * kv_ref[0, s0:s0 + CH, :]
                for t in range(1, NT):
                    acc = acc + q[t] * kv_ref[t, s0:s0 + CH, :]
                acc = acc + pltpu.roll(acc, 2 * H, 1)
                acc = acc + pltpu.roll(acc, H, 1)
                if first and r0 < DIL * w:
                    row = r0 + jax.lax.broadcasted_iota(jnp.int32, (CH, LANES), 0)
                    acc = jnp.where(row >= DIL * w, acc, -1e9 * LOG2E)
                logits.append(acc)
            m = logits[0]
            for w in range(1, W):
                m = jnp.maximum(m, logits[w])
            p = [jnp.exp2(lg - m) for lg in logits]
            den = p[0]
            for w in range(1, W):
                den = den + p[w]
            dens[c] = den
            inv = 1.0 / den
            for t in range(NT):
                acc = p[0] * kv_ref[NT + t, HALO + r0:HALO + r0 + CH, :]
                for w in range(1, W):
                    s0 = HALO + r0 - DIL * w
                    acc = acc + p[w] * kv_ref[NT + t, s0:s0 + CH, :]
                if CH >= 16:
                    atts[l][t, o0:o0 + CH, :] = (acc * inv).astype(bf16)
                elif c % 2 == 0:
                    pend[t] = acc * inv
                else:
                    both = jnp.concatenate([pend[t], acc * inv], axis=0)
                    atts[l][t, o0 - CH:o0 + CH, :] = both.astype(bf16)

    def halo(l, base):
        kvs[l][:, 0:HALO, :] = kvs[l][:, base + TS:base + TS + HALO, :]

    def oproj(l):
        return jnp.dot(_cat(atts[l], 0, NT), _cat(wo_ref, 0, NT), preferred_element_type=f32)

    def ln(x):
        return _layernorm(x).astype(bf16)

    def ll(x):
        return _layernorm(_layernorm(x)).astype(bf16)

    def up(y):
        h = jax.lax.dot_general(y, _cat(w1_ref, 0, NT), (((1,), (1,)), ((), ())),
                                preferred_element_type=f32)
        return _gelu_x2(h + b1_ref[...].astype(f32).reshape(1, -1)).astype(bf16)

    def down(h, lo=0, n=NT):
        o = jnp.dot(h, _cat(w2_ref, lo, n), preferred_element_type=f32) * 0.5
        return o + b2_ref[...].astype(f32).reshape(1, -1)[:, lo * LANES:(lo + n) * LANES]

    def put_xn(v):
        for t in range(NT):
            xn_ref[t] = v[:, t * LANES:(t + 1) * LANES]

    for cps in (x_cp[:1], wk_cp, wq_cp, wv_cp, x_cp[1:2], wo_cp, b_cp, w1_cp, w2_cp, x_cp[2:]):
        start(cps)
    never_ref[...] = jnp.zeros((1, LANES), jnp.int32)
    kv0_ref[:, 0:HALO, :] = jnp.zeros((2 * NT, HALO, LANES), f32)
    kv1_ref[:, 0:HALO, :] = jnp.zeros((2 * NT, HALO, LANES), f32)

    wait(x_cp[:1])
    xn0 = ln(x_ref[0].astype(f32))
    wait(wk_cp)
    permute_cols(1)
    proj(xn0, 1, 0, 0, 0, 2)
    wait(wq_cp)
    permute_cols(0)
    proj(xn0, 1, 0, 0, 2, 2)
    proj(xn0, 0, 0, 0, 0, 2)
    wait(wv_cp + x_cp[1:2])
    permute_cols(2)
    proj(xn0, 0, 0, 0, 2, 2)
    xn1 = ln(x_ref[1].astype(f32))
    proj(xn0, 2, 0, 0, 0, 2)
    wait(wo_cp)
    proj(xn0, 2, 0, 0, 2, 2)
    permute_rows()
    proj(xn1, 1, 0, TS)
    proj(xn1, 2, 0, TS)
    att(0, 0, True, CH=16, NB=0)
    xb_ref[...] = x_ref[0].astype(f32) + oproj(0)
    proj(xn1, 0, 0, TS)
    y = ll(xb_ref[...])
    wait(b_cp + w1_cp + w2_cp + x_cp[2:3])
    h = up(y)
    att(0, TS, False)
    halo(0, TS)
    xb_ref[...] = xb_ref[...] + down(h)
    xa_ref[...] = x_ref[1].astype(f32) + oproj(0)
    qkv(ln(xb_ref[...]), 1)
    h = up(ll(xa_ref[...]))
    att(1, 0, True)
    halo(1, 0)
    xa_ref[...] = xa_ref[...] + down(h)
    xb_ref[...] = xb_ref[...] + oproj(1)
    put_xn(ln(x_ref[2].astype(f32)))
    wait(x_cp[3:])

    def body(j, carry):
        qkv(_cat(xn_ref, 0, NT), 0)
        h = up(ll(xb_ref[...]))
        att(0, 0, False)
        halo(0, 0)
        o_ref[j - 2] = (xb_ref[...] + down(h)).astype(bf16)
        xn = ln(xa_ref[...])
        xb_ref[...] = xa_ref[...]
        xa_ref[...] = x_ref[j].astype(f32) + oproj(0)
        qkv(xn, 1)
        h = up(ll(xa_ref[...]))
        att(1, 0, False)
        halo(1, 0)
        xa_ref[...] = xa_ref[...] + down(h)
        nxt = jnp.where(j + 1 < NBLK,
                        x_ref[jnp.minimum(j + 1, NBLK - 1)].astype(f32), xa_ref[...])
        put_xn(ln(nxt))
        xb_ref[...] = xb_ref[...] + oproj(1)
        o_copy(j - 2).start()
        return carry

    jax.lax.fori_loop(2, NBLK, body, 0)

    HD = D // 2
    qkv(_cat(xn_ref, 0, NT), 1)
    h = up(ll(xb_ref[...]))
    att(1, 0, False)
    o_ref[NBLK - 2, :, :HD] = (xb_ref[:, :HD] + down(h, 0, NT // 2)).astype(bf16)
    xa_ref[...] = xa_ref[...] + oproj(1)
    o_ref[NBLK - 2, :, HD:] = (xb_ref[:, HD:] + down(h, NT // 2, NT // 2)).astype(bf16)
    h = up(ll(xa_ref[...]))
    o_copy(NBLK - 2).start()
    for t in range(NT):
        cs = slice(t * LANES, (t + 1) * LANES)
        o_ref[NBLK - 1, :, cs] = (xa_ref[:, cs] + down(h, t, 1)).astype(bf16)
        o_last[t].start()
    for i in range(NBLK - 1):
        o_copy(i).wait()
    wait(o_last)


@jax.jit
def pallas_interleave_layers__sliding_local_dilated__mixer_channel_mlp__prompt_kernel(
    A_x: jax.Array,
    A_wqkv: jax.Array,
    A_wo: jax.Array,
    B_x: jax.Array,
    B_w1: jax.Array,
    B_b1: jax.Array,
    B_w2: jax.Array,
    B_b2: jax.Array,
):
    B, S, D = A_x.shape
    F = B_w1.shape[1]
    assert B == 1 and D == 4 * LANES and S % TS == 0 and S // TS >= 3
    NT = D // LANES
    NBLK = S // TS
    f32 = jnp.float32
    bf16 = jnp.bfloat16

    hbm = pl.BlockSpec(memory_space=pl.ANY)
    out = pl.pallas_call(
        functools.partial(_kernel, D=D, NBLK=NBLK),
        in_specs=[hbm] * 7,
        out_specs=hbm,
        out_shape=jax.ShapeDtypeStruct((S, D), A_x.dtype),
        scratch_shapes=[
            pltpu.VMEM((2 * NT, 2 * TS + HALO, LANES), f32),
            pltpu.VMEM((2 * NT, TS + HALO, LANES), f32),
            pltpu.VMEM((NT, 2 * TS, LANES), f32),
            pltpu.VMEM((NT, TS, LANES), f32),
            pltpu.VMEM((NT, TS, LANES), bf16),
            pltpu.VMEM((NT, TS, LANES), bf16),
            pltpu.VMEM((TS, D), f32),
            pltpu.VMEM((TS, D), f32),
            pltpu.VMEM((NT, TS, LANES), bf16),
            pltpu.VMEM((3 * NT, D, LANES), bf16),
            pltpu.VMEM((NT, D, LANES), bf16),
            pltpu.VMEM((NT, H * WO_PITCH, LANES), f32),
            pltpu.VMEM((NBLK, TS, D), bf16),
            pltpu.VMEM((NBLK, TS, D), bf16),
            pltpu.VMEM((3 * NT, D, LANES), bf16),
            pltpu.VMEM((D, D), bf16),
            pltpu.VMEM((NT, F, LANES), bf16),
            pltpu.VMEM((NT, F, LANES), bf16),
            pltpu.VMEM((F,), bf16),
            pltpu.VMEM((D,), bf16),
            pltpu.VMEM((1, LANES), jnp.int32),
            pltpu.SemaphoreType.DMA((5 * NT + 3 + NBLK,)),
            pltpu.SemaphoreType.DMA((NBLK - 1 + NT,)),
        ],
        compiler_params=pltpu.CompilerParams(
            vmem_limit_bytes=100 * 1024 * 1024,
        ),
    )(A_x.reshape(S, D), A_wqkv, A_wo, B_w1.T, B_b1, B_w2, B_b2)
    return out.reshape(B, S, D)
```

```python
import functools
import math

import jax
import jax.numpy as jnp
import jax.experimental.pallas as pl
import jax.experimental.pallas.tpu as pltpu

H = 32
W = 8
DIL = 2
HALO = 16
EPS = 1e-5
LANES = 128
TS = 256
WO_PITCH = 17
NSEM = 3
LOG2E = math.log2(math.e)


def _gelu_x2(x):
    c = math.sqrt(2.0 / math.pi)
    inner = x * (c + (c * 0.044715) * (x * x))
    return x + x * jnp.tanh(inner)


def _cat(ref, lo, n):
    if ref.dtype == jnp.uint32:
        return jnp.concatenate(
            [pltpu.bitcast(ref[lo + t], jnp.bfloat16) for t in range(n)], axis=1)
    return jnp.concatenate([ref[lo + t] for t in range(n)], axis=1)


def _kernel(x_hbm, wqkv_hbm, wo_hbm, w1_hbm, b1_hbm, w2_hbm, b2_hbm, o_hbm,
            kv0_ref, kv1_ref, q0_ref, q1_ref, att0_ref, att1_ref,
            xa_ref, xb_ref, y_ref, wqkv_ref, wo_ref, tmp_ref,
            x_ref, o_ref, wqkv_in, wo_in, w1_ref, w2_ref, b1_ref, b2_ref,
            never_ref, sem, *, D, NBLK):
    NT = D // LANES
    Dh = D // H
    qscale = (Dh ** -0.5) * LOG2E
    f32 = jnp.float32
    bf16 = jnp.bfloat16

    def x_copy(lo, n, s):
        return pltpu.make_async_copy(x_hbm.at[pl.ds(lo, n)], x_ref.at[pl.ds(lo, n)], s)

    def w_copy(j, s):
        return pltpu.make_async_copy(wqkv_hbm.at[:, pl.ds(j * D, D)], wqkv_in.at[j], s)

    groups = [
        lambda s: [x_copy(0, 1, s)],
        lambda s: [w_copy(1, s)],
        lambda s: [w_copy(0, s)],
        lambda s: [w_copy(2, s), x_copy(1, 1, s)],
        lambda s: [pltpu.make_async_copy(wo_hbm, wo_in, s), x_copy(2, 1, s)],
        lambda s: [pltpu.make_async_copy(src, dst, s) for src, dst in (
            (b1_hbm, b1_ref), (b2_hbm, b2_ref), (w1_hbm, w1_ref), (w2_hbm, w2_ref))],
        lambda s: [x_copy(3, NBLK - 3, s)],
    ]
    groups = [g(sem.at[i % NSEM]) for i, g in enumerate(groups)]

    def start(g):
        for c in groups[g]:
            c.start()

    def wait(g):
        for c in groups[g]:
            c.wait()
        if g + NSEM < len(groups):
            start(g + NSEM)

    def o_copy(i):
        return pltpu.make_async_copy(o_ref.at[i], o_hbm.at[pl.ds(i * TS, TS), :], sem.at[1])

    o_last = [pltpu.make_async_copy(
        o_ref.at[NBLK - 1, :, pl.ds(t * LANES, LANES)],
        o_hbm.at[pl.ds((NBLK - 1) * TS, TS), pl.ds(t * LANES, LANES)],
        sem.at[1]) for t in range(NT)]

    kvs = (kv0_ref, kv1_ref)
    qs = (q0_ref, q1_ref)
    atts = (att0_ref, att1_ref)

    def permute_cols(j):
        lane = jax.lax.broadcasted_iota(jnp.int32, (1, LANES), 1)
        pgrp = (lane % 16) // 4
        a = []
        for i in range(NT):
            ai = pltpu.bitcast(wqkv_in[j, :, i * LANES:(i + 1) * LANES], jnp.uint32)
            a.append(pltpu.roll(ai, 4 * i, 1) if i else ai)
        for t in range(NT):
            c = a[(0 - t) % 4]
            for p in range(1, 4):
                c = jnp.where(pgrp == p, a[(p - t) % 4], c)
            l2 = jax.lax.broadcasted_iota(jnp.int32, c.shape, 1)
            hh = l2 % H
            src = ((hh % 8) * 16 + 4 * t + l2 // H + 4 * (hh // 8)) & (LANES - 1)
            wqkv_ref[j * NT + t] = jnp.take_along_axis(c, src, axis=1)

    def permute_rows():
        for t in range(NT):
            for h in range(H):
                tmp_ref[t, h * WO_PITCH:h * WO_PITCH + Dh, :] = (
                    wo_in[h * Dh:(h + 1) * Dh, t * LANES:(t + 1) * LANES].astype(f32))
        for d in range(Dh):
            for t in range(NT):
                wo_ref[t, d * H // 2:(d + 1) * H // 2, :] = pltpu.bitcast(
                    tmp_ref[t, pl.ds(d, H, stride=WO_PITCH), :].astype(bf16), jnp.uint32)

    Q, K, V = 0, 1, 2

    def proj(xn, j, s, base=0, t0=0, nt=NT):
        r = jnp.dot(xn, _cat(wqkv_ref, j * NT + t0, nt), preferred_element_type=f32)
        for t in range(t0, t0 + nt):
            rt = r[:, (t - t0) * LANES:(t - t0 + 1) * LANES]
            if j == Q:
                qs[s][t, base:base + TS, :] = rt
            else:
                kvs[s][(j - 1) * NT + t, HALO + base:HALO + base + TS, :] = rt

    def qkv(xn, s):
        for j in (K, V, Q):
            proj(xn, j, s)

    def att(s, base=0, first=False, CH=8, NB=3):
        kv_ref = kvs[s]
        never = jnp.broadcast_to(never_ref[...], (CH, LANES)) > 0
        dens = {}
        pend = {}
        for c in range(TS // CH):
            o0 = c * CH
            r0 = base + o0
            sc = jnp.where(never, dens[c - NB], qscale) if c >= NB else qscale
            q = [qs[s][t, r0:r0 + CH, :] * sc for t in range(NT)]
            logits = []
            for w in range(W):
                s0 = HALO + r0 - DIL * w
                acc = q[0] * kv_ref[0, s0:s0 + CH, :]
                for t in range(1, NT):
                    acc = acc + q[t] * kv_ref[t, s0:s0 + CH, :]
                acc = acc + pltpu.roll(acc, 2 * H, 1)
                acc = acc + pltpu.roll(acc, H, 1)
                if first and o0 < DIL * w:
                    row = o0 + jax.lax.broadcasted_iota(jnp.int32, (CH, LANES), 0)
                    acc = jnp.where(row >= DIL * w, acc, -1e9 * LOG2E)
                logits.append(acc)
            m = logits[0]
            for w in range(1, W):
                m = jnp.maximum(m, logits[w])
            p = [jnp.exp2(lg - m) for lg in logits]
            den = p[0]
            for w in range(1, W):
                den = den + p[w]
            dens[c] = den
            inv = 1.0 / den
            for t in range(NT):
                acc = p[0] * kv_ref[NT + t, HALO + r0:HALO + r0 + CH, :]
                for w in range(1, W):
                    s0 = HALO + r0 - DIL * w
                    acc = acc + p[w] * kv_ref[NT + t, s0:s0 + CH, :]
                if c % 2 == 0:
                    pend[t] = acc * inv
                else:
                    both = jnp.concatenate([pend[t], acc * inv], axis=0)
                    atts[s][t, o0 - CH:o0 + CH, :] = both.astype(bf16)

    def halo(s, base=0):
        kvs[s][:, 0:HALO, :] = kvs[s][:, base + TS:base + TS + HALO, :]

    def oproj(s):
        return jnp.dot(_cat(atts[s], 0, NT), _cat(wo_ref, 0, NT), preferred_element_type=f32)

    def norm(x, times, pace):
        RC, NB = pace if pace else (TS, 1)
        never = jnp.broadcast_to(never_ref[:, 0:1], (RC, 1)) > 0
        outs, rs = [], []
        for c in range(TS // RC):
            y = x[c * RC:(c + 1) * RC]
            for i in range(times):
                paced = i == 0 and c >= NB
                inv_d = jnp.where(never, rs[c - NB], 1.0 / D) if paced else 1.0 / D
                yc = y - jnp.sum(y, axis=-1, keepdims=True) * inv_d
                r = jax.lax.rsqrt(jnp.mean(yc * yc, axis=-1, keepdims=True) + EPS)
                y = yc * r
            outs.append(y.astype(bf16))
            rs.append(r)
        return jnp.concatenate(outs, axis=0)

    def ln(x, pace=(16, 5)):
        return norm(x, 1, pace)

    def ll(x, pace=(16, 5)):
        return norm(x, 2, pace)

    def up(y):
        h = jax.lax.dot_general(y, w1_ref[...], (((1,), (1,)), ((), ())),
                                preferred_element_type=f32)
        return _gelu_x2(h + b1_ref[...].astype(f32).reshape(1, -1)).astype(bf16)

    def down(h, lo=0, n=NT):
        o = jnp.dot(h, w2_ref[:, lo * LANES:(lo + n) * LANES],
                    preferred_element_type=f32) * 0.5
        return o + b2_ref[...].astype(f32).reshape(1, -1)[:, lo * LANES:(lo + n) * LANES]

    def put_y(v):
        for t in range(NT):
            y_ref[t] = v[:, t * LANES:(t + 1) * LANES]

    for g in range(NSEM):
        start(g)
    B0 = TS + HALO
    B1 = B0 + TS
    never_ref[...] = jnp.zeros((1, LANES), jnp.int32)
    kv0_ref[:, B0:B0 + HALO, :] = jnp.zeros((2 * NT, HALO, LANES), f32)
    kv1_ref[:, 0:HALO, :] = jnp.zeros((2 * NT, HALO, LANES), f32)

    wait(0)
    xn0 = ln(x_ref[0].astype(f32), None)
    wait(1)
    permute_cols(K)
    proj(xn0, K, 0, B0, 0, 2)
    wait(2)
    permute_cols(Q)
    proj(xn0, K, 0, B0, 2, 2)
    proj(xn0, Q, 0, B0, 0, 2)
    wait(3)
    permute_cols(V)
    proj(xn0, Q, 0, B0, 2, 2)
    xn1 = ln(x_ref[1].astype(f32), None)
    proj(xn0, V, 0, B0)
    wait(4)
    permute_rows()
    proj(xn1, K, 0, B1)
    proj(xn1, V, 0, B1)
    halo(0, B1)
    proj(xn1, Q, 0, B1)
    att(0, B0, first=True, NB=5)
    xn2 = ln(x_ref[2].astype(f32))
    xb_ref[...] = x_ref[0].astype(f32) + oproj(0)
    proj(xn2, K, 0)
    y = ll(xb_ref[...], None)
    wait(5)
    h = up(y)
    att(0, B1)
    xb_ref[...] = xb_ref[...] + down(h)
    xa_ref[...] = x_ref[1].astype(f32) + oproj(0)
    qkv(ln(xb_ref[...], (64, 2)), 1)
    h = up(ll(xa_ref[...]))
    att(1, first=True)
    halo(1)
    xa_ref[...] = xa_ref[...] + down(h)
    xb_ref[...] = xb_ref[...] + oproj(1)
    proj(xn2, V, 0)
    proj(xn2, Q, 0)
    put_y(ll(xb_ref[...]))
    wait(6)

    def body(j, carry):
        h = up(_cat(y_ref, 0, NT))
        att(0)
        halo(0)
        o_ref[j - 2] = (xb_ref[...] + down(h)).astype(bf16)
        xn = ln(xa_ref[...])
        xb_ref[...] = xa_ref[...]
        xa_ref[...] = x_ref[j].astype(f32) + oproj(0)
        qkv(xn, 1)
        h = up(ll(xa_ref[...]))
        att(1)
        halo(1)
        xa_ref[...] = xa_ref[...] + down(h)
        nxt = jnp.where(j + 1 < NBLK,
                        x_ref[jnp.minimum(j + 1, NBLK - 1)].astype(f32), xa_ref[...])
        xn = ln(nxt)
        xb_ref[...] = xb_ref[...] + oproj(1)
        qkv(xn, 0)
        put_y(ll(xb_ref[...]))
        o_copy(j - 2).start()
        return carry

    jax.lax.fori_loop(2, NBLK, body, 0)

    HD = D // 2
    kv0_ref[:, 0:HALO, :] = kv1_ref[:, 0:HALO, :]
    h = up(_cat(y_ref, 0, NT))
    att(0)
    o_ref[NBLK - 2, :, :HD] = (xb_ref[:, :HD] + down(h, 0, NT // 2)).astype(bf16)
    xa_ref[...] = xa_ref[...] + oproj(0)
    o_ref[NBLK - 2, :, HD:] = (xb_ref[:, HD:] + down(h, NT // 2, NT // 2)).astype(bf16)
    h = up(ll(xa_ref[...], (64, 2)))
    o_copy(NBLK - 2).start()
    for t in range(NT):
        cs = slice(t * LANES, (t + 1) * LANES)
        o_ref[NBLK - 1, :, cs] = (xa_ref[:, cs] + down(h, t, 1)).astype(bf16)
        o_last[t].start()
    for i in range(NBLK - 1):
        o_copy(i).wait()
    for c in o_last:
        c.wait()


@jax.jit
def pallas_interleave_layers__sliding_local_dilated__mixer_channel_mlp__prompt_kernel(
    A_x: jax.Array,
    A_wqkv: jax.Array,
    A_wo: jax.Array,
    B_x: jax.Array,
    B_w1: jax.Array,
    B_b1: jax.Array,
    B_w2: jax.Array,
    B_b2: jax.Array,
):
    B, S, D = A_x.shape
    F = B_w1.shape[1]
    assert B == 1 and D == 4 * LANES and S % TS == 0 and S // TS >= 4
    NT = D // LANES
    NBLK = S // TS
    f32 = jnp.float32
    bf16 = jnp.bfloat16

    hbm = pl.BlockSpec(memory_space=pl.ANY)
    out = pl.pallas_call(
        functools.partial(_kernel, D=D, NBLK=NBLK),
        in_specs=[hbm] * 7,
        out_specs=hbm,
        out_shape=jax.ShapeDtypeStruct((S, D), A_x.dtype),
        scratch_shapes=[
            pltpu.VMEM((2 * NT, 3 * TS + 2 * HALO + 8, LANES), f32),
            pltpu.VMEM((2 * NT, TS + HALO, LANES), f32),
            pltpu.VMEM((NT, 3 * TS + HALO, LANES), f32),
            pltpu.VMEM((NT, TS, LANES), f32),
            pltpu.VMEM((NT, TS, LANES), bf16),
            pltpu.VMEM((NT, TS, LANES), bf16),
            pltpu.VMEM((TS, D), f32),
            pltpu.VMEM((TS, D), f32),
            pltpu.VMEM((NT, TS, LANES), bf16),
            pltpu.VMEM((3 * NT, D // 2, LANES), jnp.uint32),
            pltpu.VMEM((NT, D // 2, LANES), jnp.uint32),
            pltpu.VMEM((NT, H * WO_PITCH, LANES), f32),
            pltpu.VMEM((NBLK, TS, D), bf16),
            pltpu.VMEM((NBLK, TS, D), bf16),
            pltpu.VMEM((3, D, D), bf16),
            pltpu.VMEM((D, D), bf16),
            pltpu.VMEM((F, D), bf16),
            pltpu.VMEM((F, D), bf16),
            pltpu.VMEM((F,), bf16),
            pltpu.VMEM((D,), bf16),
            pltpu.VMEM((1, LANES), jnp.int32),
            pltpu.SemaphoreType.DMA((NSEM,)),
        ],
        compiler_params=pltpu.CompilerParams(
            vmem_limit_bytes=100 * 1024 * 1024,
        ),
    )(A_x.reshape(NBLK, TS, D), A_wqkv, A_wo, B_w1.T, B_b1, B_w2, B_b2)
    return out.reshape(B, S, D)
```

```python
import functools
import math

import jax
import jax.numpy as jnp
import jax.experimental.pallas as pl
import jax.experimental.pallas.tpu as pltpu

H = 32
W = 8
DIL = 2
HALO = 16
EPS = 1e-5
LANES = 128
TS = 256
WO_PITCH = 17
NSEM = 3
LOG2E = math.log2(math.e)


def _layernorm(x):
    xc = x - jnp.sum(x, axis=-1, keepdims=True) * (1.0 / x.shape[-1])
    v = jnp.mean(xc * xc, axis=-1, keepdims=True)
    return xc * jax.lax.rsqrt(v + EPS)


def _gelu_x2(x):
    c = math.sqrt(2.0 / math.pi)
    inner = x * (c + (c * 0.044715) * (x * x))
    return x + x * jnp.tanh(inner)


def _cat(ref, lo, n):
    if ref.dtype == jnp.uint32:
        return jnp.concatenate(
            [pltpu.bitcast(ref[lo + t], jnp.bfloat16) for t in range(n)], axis=1)
    return jnp.concatenate([ref[lo + t] for t in range(n)], axis=1)


def _kernel(x_hbm, wqkv_hbm, wo_hbm, w1_hbm, b1_hbm, w2_hbm, b2_hbm, o_hbm,
            kv0_ref, kv1_ref, q0_ref, q1_ref, att0_ref, att1_ref,
            xa_ref, xb_ref, y_ref, wqkv_ref, wo_ref, tmp_ref,
            x_ref, o_ref, wqkv_in, wo_in, w1_ref, w2_ref, b1_ref, b2_ref,
            never_ref, sem, *, D, NBLK):
    NT = D // LANES
    Dh = D // H
    qscale = (Dh ** -0.5) * LOG2E
    f32 = jnp.float32
    bf16 = jnp.bfloat16

    def x_copy(lo, n, s):
        return pltpu.make_async_copy(x_hbm.at[pl.ds(lo, n)], x_ref.at[pl.ds(lo, n)], s)

    def w_copy(j, s):
        return pltpu.make_async_copy(wqkv_hbm.at[:, pl.ds(j * D, D)], wqkv_in.at[j], s)

    groups = [
        lambda s: [x_copy(0, 1, s)],
        lambda s: [w_copy(1, s)],
        lambda s: [w_copy(0, s)],
        lambda s: [w_copy(2, s), x_copy(1, 1, s)],
        lambda s: [pltpu.make_async_copy(wo_hbm, wo_in, s), x_copy(2, 1, s)],
        lambda s: [pltpu.make_async_copy(src, dst, s) for src, dst in (
            (b1_hbm, b1_ref), (b2_hbm, b2_ref), (w1_hbm, w1_ref), (w2_hbm, w2_ref))],
        lambda s: [x_copy(3, NBLK - 3, s)],
    ]
    groups = [g(sem.at[i % NSEM]) for i, g in enumerate(groups)]

    def start(g):
        for c in groups[g]:
            c.start()

    def wait(g):
        for c in groups[g]:
            c.wait()
        if g + NSEM < len(groups):
            start(g + NSEM)

    def o_copy(i):
        return pltpu.make_async_copy(o_ref.at[i], o_hbm.at[pl.ds(i * TS, TS), :], sem.at[1])

    o_last = [pltpu.make_async_copy(
        o_ref.at[NBLK - 1, :, pl.ds(t * LANES, LANES)],
        o_hbm.at[pl.ds((NBLK - 1) * TS, TS), pl.ds(t * LANES, LANES)],
        sem.at[1]) for t in range(NT)]

    kvs = (kv0_ref, kv1_ref)
    qs = (q0_ref, q1_ref)
    atts = (att0_ref, att1_ref)

    def permute_cols(j):
        lane = jax.lax.broadcasted_iota(jnp.int32, (1, LANES), 1)
        pgrp = (lane % 16) // 4
        a = []
        for i in range(NT):
            ai = pltpu.bitcast(wqkv_in[j, :, i * LANES:(i + 1) * LANES], jnp.uint32)
            a.append(pltpu.roll(ai, 4 * i, 1) if i else ai)
        for t in range(NT):
            c = a[(0 - t) % 4]
            for p in range(1, 4):
                c = jnp.where(pgrp == p, a[(p - t) % 4], c)
            l2 = jax.lax.broadcasted_iota(jnp.int32, c.shape, 1)
            hh = l2 % H
            src = ((hh % 8) * 16 + 4 * t + l2 // H + 4 * (hh // 8)) & (LANES - 1)
            wqkv_ref[j * NT + t] = jnp.take_along_axis(c, src, axis=1)

    def permute_rows():
        for t in range(NT):
            for h in range(H):
                tmp_ref[t, h * WO_PITCH:h * WO_PITCH + Dh, :] = (
                    wo_in[h * Dh:(h + 1) * Dh, t * LANES:(t + 1) * LANES].astype(f32))
        for d in range(Dh):
            for t in range(NT):
                wo_ref[t, d * H // 2:(d + 1) * H // 2, :] = pltpu.bitcast(
                    tmp_ref[t, pl.ds(d, H, stride=WO_PITCH), :].astype(bf16), jnp.uint32)

    Q, K, V = 0, 1, 2

    def proj(xn, j, s, base=0, t0=0, nt=NT):
        r = jnp.dot(xn, _cat(wqkv_ref, j * NT + t0, nt), preferred_element_type=f32)
        for t in range(t0, t0 + nt):
            rt = r[:, (t - t0) * LANES:(t - t0 + 1) * LANES]
            if j == Q:
                qs[s][t, base:base + TS, :] = rt
            else:
                kvs[s][(j - 1) * NT + t, HALO + base:HALO + base + TS, :] = rt

    def qkv(xn, s):
        for j in (K, V, Q):
            proj(xn, j, s)

    def att(s, base=0, first=False, CH=8, NB=3):
        kv_ref = kvs[s]
        never = jnp.broadcast_to(never_ref[...], (CH, LANES)) > 0
        dens = {}
        pend = {}
        for c in range(TS // CH):
            o0 = c * CH
            r0 = base + o0
            sc = jnp.where(never, dens[c - NB], qscale) if c >= NB else qscale
            q = [qs[s][t, r0:r0 + CH, :] * sc for t in range(NT)]
            logits = []
            for w in range(W):
                s0 = HALO + r0 - DIL * w
                acc = q[0] * kv_ref[0, s0:s0 + CH, :]
                for t in range(1, NT):
                    acc = acc + q[t] * kv_ref[t, s0:s0 + CH, :]
                acc = acc + pltpu.roll(acc, 2 * H, 1)
                acc = acc + pltpu.roll(acc, H, 1)
                if first and o0 < DIL * w:
                    row = o0 + jax.lax.broadcasted_iota(jnp.int32, (CH, LANES), 0)
                    acc = jnp.where(row >= DIL * w, acc, -1e9 * LOG2E)
                logits.append(acc)
            m = logits[0]
            for w in range(1, W):
                m = jnp.maximum(m, logits[w])
            p = [jnp.exp2(lg - m) for lg in logits]
            den = p[0]
            for w in range(1, W):
                den = den + p[w]
            dens[c] = den
            inv = 1.0 / den
            for t in range(NT):
                acc = p[0] * kv_ref[NT + t, HALO + r0:HALO + r0 + CH, :]
                for w in range(1, W):
                    s0 = HALO + r0 - DIL * w
                    acc = acc + p[w] * kv_ref[NT + t, s0:s0 + CH, :]
                if c % 2 == 0:
                    pend[t] = acc * inv
                else:
                    both = jnp.concatenate([pend[t], acc * inv], axis=0)
                    atts[s][t, o0 - CH:o0 + CH, :] = both.astype(bf16)

    def halo(s, base=0):
        kvs[s][:, 0:HALO, :] = kvs[s][:, base + TS:base + TS + HALO, :]

    def oproj(s):
        return jnp.dot(_cat(atts[s], 0, NT), _cat(wo_ref, 0, NT), preferred_element_type=f32)

    def ln(x):
        return _layernorm(x).astype(bf16)

    def ll(x):
        return _layernorm(_layernorm(x)).astype(bf16)

    def up(y):
        nt = (((1,), (1,)), ((), ()))
        F = w1_ref.shape[0]
        FM = F // LANES * LANES
        hr = jax.lax.dot_general(w1_ref[FM:, :], y, nt, preferred_element_type=f32).T
        h = jax.lax.dot_general(y, w1_ref[:FM, :], nt, preferred_element_type=f32)
        h = jnp.concatenate([h, hr], axis=1)
        return _gelu_x2(h + b1_ref[...].astype(f32).reshape(1, -1)).astype(bf16)

    def down(h, lo=0, n=NT):
        o = jnp.dot(h, w2_ref[:, lo * LANES:(lo + n) * LANES],
                    preferred_element_type=f32) * 0.5
        return o + b2_ref[...].astype(f32).reshape(1, -1)[:, lo * LANES:(lo + n) * LANES]

    def put_y(v):
        for t in range(NT):
            y_ref[t] = v[:, t * LANES:(t + 1) * LANES]

    for g in range(NSEM):
        start(g)
    B0 = TS + HALO
    B1 = B0 + TS
    never_ref[...] = jnp.zeros((1, LANES), jnp.int32)
    kv0_ref[:, B0:B0 + HALO, :] = jnp.zeros((2 * NT, HALO, LANES), f32)
    kv1_ref[:, 0:HALO, :] = jnp.zeros((2 * NT, HALO, LANES), f32)

    wait(0)
    xn0 = ln(x_ref[0].astype(f32))
    wait(1)
    permute_cols(K)
    proj(xn0, K, 0, B0, 0, 2)
    wait(2)
    permute_cols(Q)
    proj(xn0, K, 0, B0, 2, 2)
    proj(xn0, Q, 0, B0, 0, 2)
    wait(3)
    permute_cols(V)
    proj(xn0, Q, 0, B0, 2, 2)
    xn1 = ln(x_ref[1].astype(f32))
    proj(xn0, V, 0, B0)
    wait(4)
    permute_rows()
    proj(xn1, K, 0, B1)
    proj(xn1, V, 0, B1)
    halo(0, B1)
    proj(xn1, Q, 0, B1)
    att(0, B0, first=True, NB=5)
    xn2 = ln(x_ref[2].astype(f32))
    xb_ref[...] = x_ref[0].astype(f32) + oproj(0)
    proj(xn2, K, 0)
    y = ll(xb_ref[...])
    wait(5)
    h = up(y)
    att(0, B1)
    xb_ref[...] = xb_ref[...] + down(h)
    xa_ref[...] = x_ref[1].astype(f32) + oproj(0)
    qkv(ln(xb_ref[...]), 1)
    h = up(ll(xa_ref[...]))
    att(1, first=True)
    halo(1)
    xa_ref[...] = xa_ref[...] + down(h)
    xb_ref[...] = xb_ref[...] + oproj(1)
    proj(xn2, V, 0)
    proj(xn2, Q, 0)
    put_y(ll(xb_ref[...]))
    wait(6)

    def body(j, carry):
        h = up(_cat(y_ref, 0, NT))
        att(0)
        halo(0)
        o_ref[j - 2] = (xb_ref[...] + down(h)).astype(bf16)
        xn = ln(xa_ref[...])
        xb_ref[...] = xa_ref[...]
        xa_ref[...] = x_ref[j].astype(f32) + oproj(0)
        qkv(xn, 1)
        h = up(ll(xa_ref[...]))
        att(1)
        halo(1)
        xa_ref[...] = xa_ref[...] + down(h)
        nxt = jnp.where(j + 1 < NBLK,
                        x_ref[jnp.minimum(j + 1, NBLK - 1)].astype(f32), xa_ref[...])
        xn = ln(nxt)
        xb_ref[...] = xb_ref[...] + oproj(1)
        qkv(xn, 0)
        put_y(ll(xb_ref[...]))
        o_copy(j - 2).start()
        return carry

    jax.lax.fori_loop(2, NBLK, body, 0)

    HD = D // 2
    kv0_ref[:, 0:HALO, :] = kv1_ref[:, 0:HALO, :]
    h = up(_cat(y_ref, 0, NT))
    att(0)
    o_ref[NBLK - 2, :, :HD] = (xb_ref[:, :HD] + down(h, 0, NT // 2)).astype(bf16)
    xa_ref[...] = xa_ref[...] + oproj(0)
    o_ref[NBLK - 2, :, HD:] = (xb_ref[:, HD:] + down(h, NT // 2, NT // 2)).astype(bf16)
    h = up(ll(xa_ref[...]))
    o_copy(NBLK - 2).start()
    for t in range(NT):
        cs = slice(t * LANES, (t + 1) * LANES)
        o_ref[NBLK - 1, :, cs] = (xa_ref[:, cs] + down(h, t, 1)).astype(bf16)
        o_last[t].start()
    for i in range(NBLK - 1):
        o_copy(i).wait()
    for c in o_last:
        c.wait()


@jax.jit
def pallas_interleave_layers__sliding_local_dilated__mixer_channel_mlp__prompt_kernel(
    A_x: jax.Array,
    A_wqkv: jax.Array,
    A_wo: jax.Array,
    B_x: jax.Array,
    B_w1: jax.Array,
    B_b1: jax.Array,
    B_w2: jax.Array,
    B_b2: jax.Array,
):
    B, S, D = A_x.shape
    F = B_w1.shape[1]
    assert B == 1 and D == 4 * LANES and S % TS == 0 and S // TS >= 4
    NT = D // LANES
    NBLK = S // TS
    f32 = jnp.float32
    bf16 = jnp.bfloat16

    hbm = pl.BlockSpec(memory_space=pl.ANY)
    out = pl.pallas_call(
        functools.partial(_kernel, D=D, NBLK=NBLK),
        in_specs=[hbm] * 7,
        out_specs=hbm,
        out_shape=jax.ShapeDtypeStruct((S, D), A_x.dtype),
        scratch_shapes=[
            pltpu.VMEM((2 * NT, 3 * TS + 2 * HALO + 8, LANES), f32),
            pltpu.VMEM((2 * NT, TS + HALO, LANES), f32),
            pltpu.VMEM((NT, 3 * TS + HALO, LANES), f32),
            pltpu.VMEM((NT, TS, LANES), f32),
            pltpu.VMEM((NT, TS, LANES), bf16),
            pltpu.VMEM((NT, TS, LANES), bf16),
            pltpu.VMEM((TS, D), f32),
            pltpu.VMEM((TS, D), f32),
            pltpu.VMEM((NT, TS, LANES), bf16),
            pltpu.VMEM((3 * NT, D // 2, LANES), jnp.uint32),
            pltpu.VMEM((NT, D // 2, LANES), jnp.uint32),
            pltpu.VMEM((NT, H * WO_PITCH, LANES), f32),
            pltpu.VMEM((NBLK, TS, D), bf16),
            pltpu.VMEM((NBLK, TS, D), bf16),
            pltpu.VMEM((3, D, D), bf16),
            pltpu.VMEM((D, D), bf16),
            pltpu.VMEM((F, D), bf16),
            pltpu.VMEM((F, D), bf16),
            pltpu.VMEM((F,), bf16),
            pltpu.VMEM((D,), bf16),
            pltpu.VMEM((1, LANES), jnp.int32),
            pltpu.SemaphoreType.DMA((NSEM,)),
        ],
        compiler_params=pltpu.CompilerParams(
            vmem_limit_bytes=100 * 1024 * 1024,
        ),
    )(A_x.reshape(NBLK, TS, D), A_wqkv, A_wo, B_w1.T, B_b1, B_w2, B_b2)
    return out.reshape(B, S, D)
```

```python
import functools
import math

import jax
import jax.numpy as jnp
import jax.experimental.pallas as pl
import jax.experimental.pallas.tpu as pltpu

H = 32
W = 8
DIL = 2
HALO = 16
EPS = 1e-5
LANES = 128
TS = 256
WO_PITCH = 17
NSEM = 3
LOG2E = math.log2(math.e)


def _layernorm(x):
    xc = x - jnp.sum(x, axis=-1, keepdims=True) * (1.0 / x.shape[-1])
    v = jnp.mean(xc * xc, axis=-1, keepdims=True)
    return xc * jax.lax.rsqrt(v + EPS)


def _gelu_x2(x):
    c = math.sqrt(2.0 / math.pi)
    inner = x * (c + (c * 0.044715) * (x * x))
    return x + x * jnp.tanh(inner)


def _cat(ref, lo, n):
    if ref.dtype == jnp.uint32:
        return jnp.concatenate(
            [pltpu.bitcast(ref[lo + t], jnp.bfloat16) for t in range(n)], axis=1)
    return jnp.concatenate([ref[lo + t] for t in range(n)], axis=1)


def _kernel(x_hbm, wqkv_hbm, wo_hbm, w1_hbm, b1_hbm, w2_hbm, b2_hbm, o_hbm,
            kv0_ref, kv1_ref, q0_ref, q1_ref, att0_ref, att1_ref,
            xa_ref, xb_ref, y_ref, wqkv_ref, wo_ref, tmp_ref,
            x_ref, o_ref, wqkv_in, wo_in, w1_ref, w2_ref, b1_ref, b2_ref,
            never_ref, sem, *, D, NBLK):
    NT = D // LANES
    Dh = D // H
    qscale = (Dh ** -0.5) * LOG2E
    f32 = jnp.float32
    bf16 = jnp.bfloat16

    def x_copy(lo, n, s):
        return pltpu.make_async_copy(x_hbm.at[pl.ds(lo, n)], x_ref.at[pl.ds(lo, n)], s)

    def w_copy(j, s):
        return pltpu.make_async_copy(wqkv_hbm.at[:, pl.ds(j * D, D)], wqkv_in.at[j], s)

    groups = [
        lambda s: [x_copy(0, 1, s)],
        lambda s: [w_copy(1, s)],
        lambda s: [w_copy(0, s)],
        lambda s: [w_copy(2, s), x_copy(1, 1, s)],
        lambda s: [pltpu.make_async_copy(wo_hbm, wo_in, s), x_copy(2, 1, s)],
        lambda s: [pltpu.make_async_copy(src, dst, s) for src, dst in (
            (b1_hbm, b1_ref), (b2_hbm, b2_ref), (w1_hbm, w1_ref), (w2_hbm, w2_ref))],
        lambda s: [x_copy(3, NBLK - 3, s)],
    ]
    groups = [g(sem.at[i % NSEM]) for i, g in enumerate(groups)]

    def start(g):
        for c in groups[g]:
            c.start()

    def wait(g):
        for c in groups[g]:
            c.wait()
        if g + NSEM < len(groups):
            start(g + NSEM)

    def o_copy(i):
        return pltpu.make_async_copy(o_ref.at[i], o_hbm.at[pl.ds(i * TS, TS), :], sem.at[1])

    o_last = [pltpu.make_async_copy(
        o_ref.at[NBLK - 1, :, pl.ds(t * LANES, LANES)],
        o_hbm.at[pl.ds((NBLK - 1) * TS, TS), pl.ds(t * LANES, LANES)],
        sem.at[1]) for t in range(NT)]

    kvs = (kv0_ref, kv1_ref)
    qs = (q0_ref, q1_ref)
    atts = (att0_ref, att1_ref)

    def permute_cols(j):
        lane = jax.lax.broadcasted_iota(jnp.int32, (1, LANES), 1)
        pgrp = (lane % 16) // 4
        a = []
        for i in range(NT):
            ai = pltpu.bitcast(wqkv_in[j, :, i * LANES:(i + 1) * LANES], jnp.uint32)
            a.append(pltpu.roll(ai, 4 * i, 1) if i else ai)
        for t in range(NT):
            c = a[(0 - t) % 4]
            for p in range(1, 4):
                c = jnp.where(pgrp == p, a[(p - t) % 4], c)
            l2 = jax.lax.broadcasted_iota(jnp.int32, c.shape, 1)
            hh = l2 % H
            src = ((hh % 8) * 16 + 4 * t + l2 // H + 4 * (hh // 8)) & (LANES - 1)
            wqkv_ref[j * NT + t] = jnp.take_along_axis(c, src, axis=1)

    def permute_rows():
        for t in range(NT):
            for h in range(H):
                tmp_ref[t, h * WO_PITCH:h * WO_PITCH + Dh, :] = (
                    wo_in[h * Dh:(h + 1) * Dh, t * LANES:(t + 1) * LANES].astype(f32))
        for d in range(Dh):
            for t in range(NT):
                wo_ref[t, d * H // 2:(d + 1) * H // 2, :] = pltpu.bitcast(
                    tmp_ref[t, pl.ds(d, H, stride=WO_PITCH), :].astype(bf16), jnp.uint32)

    Q, K, V = 0, 1, 2

    def proj(xn, j, s, base=0, t0=0, nt=NT):
        r = jnp.dot(xn, _cat(wqkv_ref, j * NT + t0, nt), preferred_element_type=f32)
        for t in range(t0, t0 + nt):
            rt = r[:, (t - t0) * LANES:(t - t0 + 1) * LANES]
            if j == Q:
                qs[s][t, base:base + TS, :] = rt
            else:
                kvs[s][(j - 1) * NT + t, HALO + base:HALO + base + TS, :] = rt

    def qkv(xn, s):
        for j in (K, V, Q):
            proj(xn, j, s)

    def att(s, base=0, first=False, CH=8, NB=3):
        kv_ref = kvs[s]
        never = jnp.broadcast_to(never_ref[...], (CH, LANES)) > 0
        dens = {}
        pend = {}
        for c in range(TS // CH):
            o0 = c * CH
            r0 = base + o0
            sc = jnp.where(never, dens[c - NB], qscale) if c >= NB else qscale
            q = [qs[s][t, r0:r0 + CH, :] * sc for t in range(NT)]
            logits = []
            for w in range(W):
                s0 = HALO + r0 - DIL * w
                acc = q[0] * kv_ref[0, s0:s0 + CH, :]
                for t in range(1, NT):
                    acc = acc + q[t] * kv_ref[t, s0:s0 + CH, :]
                acc = acc + pltpu.roll(acc, 2 * H, 1)
                acc = acc + pltpu.roll(acc, H, 1)
                if first and o0 < DIL * w:
                    row = o0 + jax.lax.broadcasted_iota(jnp.int32, (CH, LANES), 0)
                    acc = jnp.where(row >= DIL * w, acc, -1e9 * LOG2E)
                logits.append(acc)
            m = logits[0]
            for w in range(1, W):
                m = jnp.maximum(m, logits[w])
            p = [jnp.exp2(lg - m) for lg in logits]
            den = p[0]
            for w in range(1, W):
                den = den + p[w]
            dens[c] = den
            inv = 1.0 / den
            for t in range(NT):
                acc = p[0] * kv_ref[NT + t, HALO + r0:HALO + r0 + CH, :]
                for w in range(1, W):
                    s0 = HALO + r0 - DIL * w
                    acc = acc + p[w] * kv_ref[NT + t, s0:s0 + CH, :]
                if c % 2 == 0:
                    pend[t] = acc * inv
                else:
                    both = jnp.concatenate([pend[t], acc * inv], axis=0)
                    atts[s][t, o0 - CH:o0 + CH, :] = both.astype(bf16)

    def halo(s, base=0):
        kvs[s][:, 0:HALO, :] = kvs[s][:, base + TS:base + TS + HALO, :]

    def oproj(s):
        return jnp.dot(_cat(atts[s], 0, NT), _cat(wo_ref, 0, NT), preferred_element_type=f32)

    def ln(x):
        return _layernorm(x).astype(bf16)

    def ll(x):
        return _layernorm(_layernorm(x)).astype(bf16)

    F = w1_ref.shape[0]
    FM = F // LANES * LANES
    nt_dims = (((1,), (1,)), ((), ()))

    def up(y, lo=0):
        hr = jax.lax.dot_general(w1_ref[FM:, :], y, nt_dims, preferred_element_type=f32).T
        h = jax.lax.dot_general(y, w1_ref[lo:FM, :], nt_dims, preferred_element_type=f32)
        h = jnp.concatenate([h, hr], axis=1)
        return _gelu_x2(h + b1_ref[...].astype(f32).reshape(1, -1)[:, lo:]).astype(bf16)

    def down(h, lo=0, n=NT):
        o = jnp.dot(h, w2_ref[:, lo * LANES:(lo + n) * LANES],
                    preferred_element_type=f32) * 0.5
        return o + b2_ref[...].astype(f32).reshape(1, -1)[:, lo * LANES:(lo + n) * LANES]

    def mlp(y):
        h1 = up(y, D)
        h0 = jax.lax.dot_general(y, w1_ref[:D, :], nt_dims, preferred_element_type=f32)
        h0 = _gelu_x2(h0 + b1_ref[...].astype(f32).reshape(1, -1)[:, :D]).astype(bf16)
        o = jnp.dot(h1, w2_ref[D:, :], preferred_element_type=f32)
        o = o + jnp.dot(h0, w2_ref[:D, :], preferred_element_type=f32)
        return o * 0.5 + b2_ref[...].astype(f32).reshape(1, -1)

    def put_y(v):
        for t in range(NT):
            y_ref[t] = v[:, t * LANES:(t + 1) * LANES]

    for g in range(NSEM):
        start(g)
    B0 = TS + HALO
    B1 = B0 + TS
    never_ref[...] = jnp.zeros((1, LANES), jnp.int32)
    kv0_ref[:, B0:B0 + HALO, :] = jnp.zeros((2 * NT, HALO, LANES), f32)
    kv1_ref[:, 0:HALO, :] = jnp.zeros((2 * NT, HALO, LANES), f32)

    wait(0)
    xn0 = ln(x_ref[0].astype(f32))
    wait(1)
    permute_cols(K)
    proj(xn0, K, 0, B0, 0, 2)
    wait(2)
    permute_cols(Q)
    proj(xn0, K, 0, B0, 2, 2)
    proj(xn0, Q, 0, B0, 0, 2)
    wait(3)
    permute_cols(V)
    proj(xn0, Q, 0, B0, 2, 2)
    xn1 = ln(x_ref[1].astype(f32))
    proj(xn0, V, 0, B0)
    wait(4)
    permute_rows()
    proj(xn1, K, 0, B1)
    proj(xn1, V, 0, B1)
    halo(0, B1)
    proj(xn1, Q, 0, B1)
    att(0, B0, first=True, NB=5)
    xn2 = ln(x_ref[2].astype(f32))
    xb_ref[...] = x_ref[0].astype(f32) + oproj(0)
    proj(xn2, K, 0)
    y = ll(xb_ref[...])
    wait(5)
    m = mlp(y)
    att(0, B1)
    xb_ref[...] = xb_ref[...] + m
    xa_ref[...] = x_ref[1].astype(f32) + oproj(0)
    qkv(ln(xb_ref[...]), 1)
    m = mlp(ll(xa_ref[...]))
    att(1, first=True)
    halo(1)
    xa_ref[...] = xa_ref[...] + m
    xb_ref[...] = xb_ref[...] + oproj(1)
    proj(xn2, V, 0)
    proj(xn2, Q, 0)
    put_y(ll(xb_ref[...]))
    wait(6)

    def body(j, carry):
        m = mlp(_cat(y_ref, 0, NT))
        att(0)
        halo(0)
        o_ref[j - 2] = (xb_ref[...] + m).astype(bf16)
        xn = ln(xa_ref[...])
        xb_ref[...] = xa_ref[...]
        xa_ref[...] = x_ref[j].astype(f32) + oproj(0)
        qkv(xn, 1)
        m = mlp(ll(xa_ref[...]))
        att(1)
        halo(1)
        xa_ref[...] = xa_ref[...] + m
        nxt = jnp.where(j + 1 < NBLK,
                        x_ref[jnp.minimum(j + 1, NBLK - 1)].astype(f32), xa_ref[...])
        xn = ln(nxt)
        xb_ref[...] = xb_ref[...] + oproj(1)
        qkv(xn, 0)
        put_y(ll(xb_ref[...]))
        o_copy(j - 2).start()
        return carry

    jax.lax.fori_loop(2, NBLK, body, 0)

    HD = D // 2
    kv0_ref[:, 0:HALO, :] = kv1_ref[:, 0:HALO, :]
    h = up(_cat(y_ref, 0, NT))
    att(0)
    o_ref[NBLK - 2, :, :HD] = (xb_ref[:, :HD] + down(h, 0, NT // 2)).astype(bf16)
    xa_ref[...] = xa_ref[...] + oproj(0)
    o_ref[NBLK - 2, :, HD:] = (xb_ref[:, HD:] + down(h, NT // 2, NT // 2)).astype(bf16)
    h = up(ll(xa_ref[...]))
    o_copy(NBLK - 2).start()
    for t in range(NT):
        cs = slice(t * LANES, (t + 1) * LANES)
        o_ref[NBLK - 1, :, cs] = (xa_ref[:, cs] + down(h, t, 1)).astype(bf16)
        o_last[t].start()
    for i in range(NBLK - 1):
        o_copy(i).wait()
    for c in o_last:
        c.wait()


@jax.jit
def pallas_interleave_layers__sliding_local_dilated__mixer_channel_mlp__prompt_kernel(
    A_x: jax.Array,
    A_wqkv: jax.Array,
    A_wo: jax.Array,
    B_x: jax.Array,
    B_w1: jax.Array,
    B_b1: jax.Array,
    B_w2: jax.Array,
    B_b2: jax.Array,
):
    B, S, D = A_x.shape
    F = B_w1.shape[1]
    assert B == 1 and D == 4 * LANES and S % TS == 0 and S // TS >= 4
    assert F % LANES != 0 and F % 16 == 0 and F > D + LANES
    NT = D // LANES
    NBLK = S // TS
    f32 = jnp.float32
    bf16 = jnp.bfloat16

    hbm = pl.BlockSpec(memory_space=pl.ANY)
    out = pl.pallas_call(
        functools.partial(_kernel, D=D, NBLK=NBLK),
        in_specs=[hbm] * 7,
        out_specs=hbm,
        out_shape=jax.ShapeDtypeStruct((S, D), A_x.dtype),
        scratch_shapes=[
            pltpu.VMEM((2 * NT, 3 * TS + 2 * HALO + 8, LANES), f32),
            pltpu.VMEM((2 * NT, TS + HALO, LANES), f32),
            pltpu.VMEM((NT, 3 * TS + HALO, LANES), f32),
            pltpu.VMEM((NT, TS, LANES), f32),
            pltpu.VMEM((NT, TS, LANES), bf16),
            pltpu.VMEM((NT, TS, LANES), bf16),
            pltpu.VMEM((TS, D), f32),
            pltpu.VMEM((TS, D), f32),
            pltpu.VMEM((NT, TS, LANES), bf16),
            pltpu.VMEM((3 * NT, D // 2, LANES), jnp.uint32),
            pltpu.VMEM((NT, D // 2, LANES), jnp.uint32),
            pltpu.VMEM((NT, H * WO_PITCH, LANES), f32),
            pltpu.VMEM((NBLK, TS, D), bf16),
            pltpu.VMEM((NBLK, TS, D), bf16),
            pltpu.VMEM((3, D, D), bf16),
            pltpu.VMEM((D, D), bf16),
            pltpu.VMEM((F, D), bf16),
            pltpu.VMEM((F, D), bf16),
            pltpu.VMEM((F,), bf16),
            pltpu.VMEM((D,), bf16),
            pltpu.VMEM((1, LANES), jnp.int32),
            pltpu.SemaphoreType.DMA((NSEM,)),
        ],
        compiler_params=pltpu.CompilerParams(
            vmem_limit_bytes=100 * 1024 * 1024,
        ),
    )(A_x.reshape(NBLK, TS, D), A_wqkv, A_wo, B_w1.T, B_b1, B_w2, B_b2)
    return out.reshape(B, S, D)
```

```python
import functools
import math

import jax
import jax.numpy as jnp
import jax.experimental.pallas as pl
import jax.experimental.pallas.tpu as pltpu

H = 32
W = 8
DIL = 2
HALO = 16
EPS = 1e-5
LANES = 128
TS = 256
WO_PITCH = 17
NSEM = 3
LOG2E = math.log2(math.e)


def _layernorm(x):
    xc = x - jnp.sum(x, axis=-1, keepdims=True) * (1.0 / x.shape[-1])
    v = jnp.mean(xc * xc, axis=-1, keepdims=True)
    return xc * jax.lax.rsqrt(v + EPS)


def _gelu_x2(x):
    c = math.sqrt(2.0 / math.pi)
    inner = x * (c + (c * 0.044715) * (x * x))
    return x + x * jnp.tanh(inner)


def _cat(ref, lo, n):
    if ref.dtype == jnp.uint32:
        return jnp.concatenate(
            [pltpu.bitcast(ref[lo + t], jnp.bfloat16) for t in range(n)], axis=1)
    return jnp.concatenate([ref[lo + t] for t in range(n)], axis=1)


def _kernel(x_hbm, wqkv_hbm, wo_hbm, w1_hbm, b1_hbm, w2_hbm, b2_hbm, o_hbm,
            kv0_ref, kv1_ref, q0_ref, q1_ref, att0_ref, att1_ref,
            xa_ref, xb_ref, y_ref, wqkv_ref, wo_ref, tmp_ref,
            x_ref, o_ref, wqkv_in, wo_in, w1_ref, w2_ref, b1_ref, b2_ref,
            never_ref, sem, *, D, NBLK):
    NT = D // LANES
    Dh = D // H
    qscale = (Dh ** -0.5) * LOG2E
    f32 = jnp.float32
    bf16 = jnp.bfloat16

    def x_copy(lo, n, s):
        return pltpu.make_async_copy(x_hbm.at[pl.ds(lo, n)], x_ref.at[pl.ds(lo, n)], s)

    def w_copy(j, s):
        return pltpu.make_async_copy(wqkv_hbm.at[:, pl.ds(j * D, D)], wqkv_in.at[j], s)

    groups = [
        lambda s: [x_copy(0, 1, s)],
        lambda s: [w_copy(1, s)],
        lambda s: [w_copy(0, s)],
        lambda s: [w_copy(2, s), x_copy(1, 1, s)],
        lambda s: [pltpu.make_async_copy(wo_hbm, wo_in, s), x_copy(2, 1, s)],
        lambda s: [pltpu.make_async_copy(src, dst, s) for src, dst in (
            (b1_hbm, b1_ref), (b2_hbm, b2_ref), (w1_hbm, w1_ref), (w2_hbm, w2_ref))],
        lambda s: [x_copy(3, NBLK - 3, s)],
    ]
    groups = [g(sem.at[i % NSEM]) for i, g in enumerate(groups)]

    def start(g):
        for c in groups[g]:
            c.start()

    def wait(g):
        for c in groups[g]:
            c.wait()
        if g + NSEM < len(groups):
            start(g + NSEM)

    def o_copy(i):
        return pltpu.make_async_copy(o_ref.at[i], o_hbm.at[pl.ds(i * TS, TS), :], sem.at[1])

    o_last = [pltpu.make_async_copy(
        o_ref.at[NBLK - 1, :, pl.ds(t * LANES, LANES)],
        o_hbm.at[pl.ds((NBLK - 1) * TS, TS), pl.ds(t * LANES, LANES)],
        sem.at[1]) for t in range(NT)]

    kvs = (kv0_ref, kv1_ref)
    qs = (q0_ref, q1_ref)
    atts = (att0_ref, att1_ref)

    def permute_cols(j):
        lane = jax.lax.broadcasted_iota(jnp.int32, (1, LANES), 1)
        pgrp = (lane % 16) // 4
        a = []
        for i in range(NT):
            ai = pltpu.bitcast(wqkv_in[j, :, i * LANES:(i + 1) * LANES], jnp.uint32)
            a.append(pltpu.roll(ai, 4 * i, 1) if i else ai)
        for t in range(NT):
            c = a[(0 - t) % 4]
            for p in range(1, 4):
                c = jnp.where(pgrp == p, a[(p - t) % 4], c)
            l2 = jax.lax.broadcasted_iota(jnp.int32, c.shape, 1)
            hh = l2 % H
            src = ((hh % 8) * 16 + 4 * t + l2 // H + 4 * (hh // 8)) & (LANES - 1)
            wqkv_ref[j * NT + t] = jnp.take_along_axis(c, src, axis=1)

    def permute_rows():
        for t in range(NT):
            for h in range(H):
                tmp_ref[t, h * WO_PITCH:h * WO_PITCH + Dh, :] = (
                    wo_in[h * Dh:(h + 1) * Dh, t * LANES:(t + 1) * LANES].astype(f32))
        for d in range(Dh):
            for t in range(NT):
                wo_ref[t, d * H // 2:(d + 1) * H // 2, :] = pltpu.bitcast(
                    tmp_ref[t, pl.ds(d, H, stride=WO_PITCH), :].astype(bf16), jnp.uint32)

    Q, K, V = 0, 1, 2

    def proj(xn, j, s, base=0, t0=0, nt=NT):
        r = jnp.dot(xn, _cat(wqkv_ref, j * NT + t0, nt), preferred_element_type=f32)
        for t in range(t0, t0 + nt):
            rt = r[:, (t - t0) * LANES:(t - t0 + 1) * LANES]
            if j == Q:
                qs[s][t, base:base + TS, :] = rt
            else:
                kvs[s][(j - 1) * NT + t, HALO + base:HALO + base + TS, :] = rt

    def qkv(xn, s):
        for j in (K, V, Q):
            proj(xn, j, s)

    def att(s, base=0, first=False, CH=8, NB=3):
        kv_ref = kvs[s]
        never = jnp.broadcast_to(never_ref[...], (CH, LANES)) > 0
        dens = {}
        pend = {}
        for c in range(TS // CH):
            o0 = c * CH
            r0 = base + o0
            sc = jnp.where(never, dens[c - NB], qscale) if c >= NB else qscale
            q = [qs[s][t, r0:r0 + CH, :] * sc for t in range(NT)]
            logits = []
            for w in range(W):
                s0 = HALO + r0 - DIL * w
                acc = q[0] * kv_ref[0, s0:s0 + CH, :]
                for t in range(1, NT):
                    acc = acc + q[t] * kv_ref[t, s0:s0 + CH, :]
                acc = acc + pltpu.roll(acc, 2 * H, 1)
                acc = acc + pltpu.roll(acc, H, 1)
                if first and o0 < DIL * w:
                    row = o0 + jax.lax.broadcasted_iota(jnp.int32, (CH, LANES), 0)
                    acc = jnp.where(row >= DIL * w, acc, -1e9 * LOG2E)
                logits.append(acc)
            m = logits[0]
            for w in range(1, W):
                m = jnp.maximum(m, logits[w])
            p = [jnp.exp2(lg - m) for lg in logits]
            den = p[0]
            for w in range(1, W):
                den = den + p[w]
            dens[c] = den
            inv = 1.0 / den
            for t in range(NT):
                acc = p[0] * kv_ref[NT + t, HALO + r0:HALO + r0 + CH, :]
                for w in range(1, W):
                    s0 = HALO + r0 - DIL * w
                    acc = acc + p[w] * kv_ref[NT + t, s0:s0 + CH, :]
                if c % 2 == 0:
                    pend[t] = acc * inv
                else:
                    both = jnp.concatenate([pend[t], acc * inv], axis=0)
                    atts[s][t, o0 - CH:o0 + CH, :] = both.astype(bf16)

    def halo(s, base=0):
        kvs[s][:, 0:HALO, :] = kvs[s][:, base + TS:base + TS + HALO, :]

    def halo_start(s, base):
        row0 = kvs[s][NT:, HALO + base:HALO + base + 1, :]
        kvs[s][NT:, base:base + HALO, :] = jnp.broadcast_to(row0, (NT, HALO, LANES))

    def oproj(s):
        return jnp.dot(_cat(atts[s], 0, NT), _cat(wo_ref, 0, NT), preferred_element_type=f32)

    def ln(x):
        return _layernorm(x).astype(bf16)

    def ll(x):
        return _layernorm(_layernorm(x)).astype(bf16)

    F = w1_ref.shape[0]
    FM = F // LANES * LANES
    nt_dims = (((1,), (1,)), ((), ()))

    def up(y, lo=0):
        hr = jax.lax.dot_general(w1_ref[FM:, :], y, nt_dims, preferred_element_type=f32).T
        h = jax.lax.dot_general(y, w1_ref[lo:FM, :], nt_dims, preferred_element_type=f32)
        h = jnp.concatenate([h, hr], axis=1)
        return _gelu_x2(h + b1_ref[...].astype(f32).reshape(1, -1)[:, lo:]).astype(bf16)

    def down(h, lo=0, n=NT):
        o = jnp.dot(h, w2_ref[:, lo * LANES:(lo + n) * LANES],
                    preferred_element_type=f32) * 0.5
        return o + b2_ref[...].astype(f32).reshape(1, -1)[:, lo * LANES:(lo + n) * LANES]

    def mlp(y):
        h1 = up(y, D)
        h0 = jax.lax.dot_general(y, w1_ref[:D, :], nt_dims, preferred_element_type=f32)
        h0 = _gelu_x2(h0 + b1_ref[...].astype(f32).reshape(1, -1)[:, :D]).astype(bf16)
        o = jnp.dot(h1, w2_ref[D:, :], preferred_element_type=f32)
        o = o + jnp.dot(h0, w2_ref[:D, :], preferred_element_type=f32)
        return o * 0.5 + b2_ref[...].astype(f32).reshape(1, -1)

    def put_y(v):
        for t in range(NT):
            y_ref[t] = v[:, t * LANES:(t + 1) * LANES]

    for g in range(NSEM):
        start(g)
    B0 = TS + HALO
    B1 = B0 + TS
    never_ref[...] = jnp.zeros((1, LANES), jnp.int32)
    kv0_ref[:NT, B0:B0 + HALO, :] = jnp.zeros((NT, HALO, LANES), f32)
    kv1_ref[:NT, 0:HALO, :] = jnp.zeros((NT, HALO, LANES), f32)

    wait(0)
    xn0 = ln(x_ref[0].astype(f32))
    wait(1)
    permute_cols(K)
    proj(xn0, K, 0, B0, 0, 2)
    wait(2)
    permute_cols(Q)
    proj(xn0, K, 0, B0, 2, 2)
    proj(xn0, Q, 0, B0, 0, 2)
    wait(3)
    permute_cols(V)
    proj(xn0, Q, 0, B0, 2, 2)
    xn1 = ln(x_ref[1].astype(f32))
    proj(xn0, V, 0, B0)
    halo_start(0, B0)
    wait(4)
    permute_rows()
    proj(xn1, K, 0, B1)
    proj(xn1, V, 0, B1)
    halo(0, B1)
    proj(xn1, Q, 0, B1)
    att(0, B0, first=True, NB=5)
    xn2 = ln(x_ref[2].astype(f32))
    xb_ref[...] = x_ref[0].astype(f32) + oproj(0)
    proj(xn2, K, 0)
    y = ll(xb_ref[...])
    wait(5)
    m = mlp(y)
    att(0, B1)
    xb_ref[...] = xb_ref[...] + m
    xa_ref[...] = x_ref[1].astype(f32) + oproj(0)
    qkv(ln(xb_ref[...]), 1)
    halo_start(1, 0)
    m = mlp(ll(xa_ref[...]))
    att(1, first=True)
    halo(1)
    xa_ref[...] = xa_ref[...] + m
    xb_ref[...] = xb_ref[...] + oproj(1)
    proj(xn2, V, 0)
    proj(xn2, Q, 0)
    put_y(ll(xb_ref[...]))
    wait(6)

    def body(j, carry):
        m = mlp(_cat(y_ref, 0, NT))
        att(0)
        halo(0)
        o_ref[j - 2] = (xb_ref[...] + m).astype(bf16)
        xn = ln(xa_ref[...])
        xb_ref[...] = xa_ref[...]
        xa_ref[...] = x_ref[j].astype(f32) + oproj(0)
        qkv(xn, 1)
        m = mlp(ll(xa_ref[...]))
        att(1)
        halo(1)
        xa_ref[...] = xa_ref[...] + m
        nxt = jnp.where(j + 1 < NBLK,
                        x_ref[jnp.minimum(j + 1, NBLK - 1)].astype(f32), xa_ref[...])
        xn = ln(nxt)
        xb_ref[...] = xb_ref[...] + oproj(1)
        qkv(xn, 0)
        put_y(ll(xb_ref[...]))
        o_copy(j - 2).start()
        return carry

    jax.lax.fori_loop(2, NBLK, body, 0)

    HD = D // 2
    kv0_ref[:, 0:HALO, :] = kv1_ref[:, 0:HALO, :]
    h = up(_cat(y_ref, 0, NT))
    att(0)
    o_ref[NBLK - 2, :, :HD] = (xb_ref[:, :HD] + down(h, 0, NT // 2)).astype(bf16)
    xa_ref[...] = xa_ref[...] + oproj(0)
    o_ref[NBLK - 2, :, HD:] = (xb_ref[:, HD:] + down(h, NT // 2, NT // 2)).astype(bf16)
    h = up(ll(xa_ref[...]))
    o_copy(NBLK - 2).start()
    for t in range(NT):
        cs = slice(t * LANES, (t + 1) * LANES)
        o_ref[NBLK - 1, :, cs] = (xa_ref[:, cs] + down(h, t, 1)).astype(bf16)
        o_last[t].start()
    for i in range(NBLK - 1):
        o_copy(i).wait()
    for c in o_last:
        c.wait()


@jax.jit
def pallas_interleave_layers__sliding_local_dilated__mixer_channel_mlp__prompt_kernel(
    A_x: jax.Array,
    A_wqkv: jax.Array,
    A_wo: jax.Array,
    B_x: jax.Array,
    B_w1: jax.Array,
    B_b1: jax.Array,
    B_w2: jax.Array,
    B_b2: jax.Array,
):
    B, S, D = A_x.shape
    F = B_w1.shape[1]
    assert B == 1 and D == 4 * LANES and S % TS == 0 and S // TS >= 4
    assert F % LANES != 0 and F % 16 == 0 and F > D + LANES
    NT = D // LANES
    NBLK = S // TS
    f32 = jnp.float32
    bf16 = jnp.bfloat16

    hbm = pl.BlockSpec(memory_space=pl.ANY)
    out = pl.pallas_call(
        functools.partial(_kernel, D=D, NBLK=NBLK),
        in_specs=[hbm] * 7,
        out_specs=hbm,
        out_shape=jax.ShapeDtypeStruct((S, D), A_x.dtype),
        scratch_shapes=[
            pltpu.VMEM((2 * NT, 3 * TS + 2 * HALO + 8, LANES), f32),
            pltpu.VMEM((2 * NT, TS + HALO, LANES), f32),
            pltpu.VMEM((NT, 3 * TS + HALO, LANES), f32),
            pltpu.VMEM((NT, TS, LANES), f32),
            pltpu.VMEM((NT, TS, LANES), bf16),
            pltpu.VMEM((NT, TS, LANES), bf16),
            pltpu.VMEM((TS, D), f32),
            pltpu.VMEM((TS, D), f32),
            pltpu.VMEM((NT, TS, LANES), bf16),
            pltpu.VMEM((3 * NT, D // 2, LANES), jnp.uint32),
            pltpu.VMEM((NT, D // 2, LANES), jnp.uint32),
            pltpu.VMEM((NT, H * WO_PITCH, LANES), f32),
            pltpu.VMEM((NBLK, TS, D), bf16),
            pltpu.VMEM((NBLK, TS, D), bf16),
            pltpu.VMEM((3, D, D), bf16),
            pltpu.VMEM((D, D), bf16),
            pltpu.VMEM((F, D), bf16),
            pltpu.VMEM((F, D), bf16),
            pltpu.VMEM((F,), bf16),
            pltpu.VMEM((D,), bf16),
            pltpu.VMEM((1, LANES), jnp.int32),
            pltpu.SemaphoreType.DMA((NSEM,)),
        ],
        compiler_params=pltpu.CompilerParams(
            vmem_limit_bytes=100 * 1024 * 1024,
        ),
    )(A_x.reshape(NBLK, TS, D), A_wqkv, A_wo, B_w1.T, B_b1, B_w2, B_b2)
    return out.reshape(B, S, D)
```

```python
import functools
import math

import jax
import jax.numpy as jnp
import jax.experimental.pallas as pl
import jax.experimental.pallas.tpu as pltpu

H = 32
W = 8
DIL = 2
HALO = 16
EPS = 1e-5
LANES = 128
TS = 256
WO_PITCH = 17
NSEM = 3
LOG2E = math.log2(math.e)


def _layernorm(x):
    xc = x - jnp.sum(x, axis=-1, keepdims=True) * (1.0 / x.shape[-1])
    v = jnp.mean(xc * xc, axis=-1, keepdims=True)
    return xc * jax.lax.rsqrt(v + EPS)


def _gelu_x2(x):
    c = math.sqrt(2.0 / math.pi)
    inner = x * (c + (c * 0.044715) * (x * x))
    return x + x * jnp.tanh(inner)


def _cat(ref, lo, n):
    if ref.dtype == jnp.uint32:
        return jnp.concatenate(
            [pltpu.bitcast(ref[lo + t], jnp.bfloat16) for t in range(n)], axis=1)
    return jnp.concatenate([ref[lo + t] for t in range(n)], axis=1)


def _kernel(x_hbm, wqkv_hbm, wo_hbm, w1_hbm, b1_hbm, w2_hbm, b2_hbm, o_hbm,
            kv0_ref, kv1_ref, q0_ref, q1_ref, att0_ref, att1_ref,
            xa_ref, xb_ref, y_ref, wqkv_ref, wo_ref, tmp_ref,
            x_ref, o_ref, wqkv_in, wo_in, w1_ref, w2_ref, b1_ref, b2_ref,
            never_ref, sem, *, D, NBLK):
    NT = D // LANES
    Dh = D // H
    qscale = (Dh ** -0.5) * LOG2E
    f32 = jnp.float32
    bf16 = jnp.bfloat16

    def x_copy(lo, n, s):
        return pltpu.make_async_copy(x_hbm.at[pl.ds(lo, n)], x_ref.at[pl.ds(lo, n)], s)

    def w_copy(j, s):
        return pltpu.make_async_copy(wqkv_hbm.at[:, pl.ds(j * D, D)], wqkv_in.at[j], s)

    groups = [
        lambda s: [x_copy(0, 1, s)],
        lambda s: [w_copy(1, s)],
        lambda s: [x_copy(1, 2, s)],
        lambda s: [w_copy(0, s)],
        lambda s: [w_copy(2, s), pltpu.make_async_copy(wo_hbm, wo_in, s)],
        lambda s: [pltpu.make_async_copy(src, dst, s) for src, dst in (
            (b1_hbm, b1_ref), (b2_hbm, b2_ref), (w1_hbm, w1_ref), (w2_hbm, w2_ref))],
        lambda s: [x_copy(3, NBLK - 3, s)],
    ]
    groups = [g(sem.at[i % NSEM]) for i, g in enumerate(groups)]

    def start(g):
        for c in groups[g]:
            c.start()

    def wait(g):
        for c in groups[g]:
            c.wait()
        if g + NSEM < len(groups):
            start(g + NSEM)

    def o_copy(i):
        return pltpu.make_async_copy(o_ref.at[i], o_hbm.at[pl.ds(i * TS, TS), :], sem.at[1])

    o_last = [pltpu.make_async_copy(
        o_ref.at[NBLK - 1, :, pl.ds(t * LANES, LANES)],
        o_hbm.at[pl.ds((NBLK - 1) * TS, TS), pl.ds(t * LANES, LANES)],
        sem.at[1]) for t in range(NT)]

    kvs = (kv0_ref, kv1_ref)
    qs = (q0_ref, q1_ref)
    atts = (att0_ref, att1_ref)

    def permute_cols(j):
        lane = jax.lax.broadcasted_iota(jnp.int32, (1, LANES), 1)
        pgrp = (lane % 16) // 4
        a = []
        for i in range(NT):
            ai = pltpu.bitcast(wqkv_in[j, :, i * LANES:(i + 1) * LANES], jnp.uint32)
            a.append(pltpu.roll(ai, 4 * i, 1) if i else ai)
        for t in range(NT):
            c = a[(0 - t) % 4]
            for p in range(1, 4):
                c = jnp.where(pgrp == p, a[(p - t) % 4], c)
            l2 = jax.lax.broadcasted_iota(jnp.int32, c.shape, 1)
            hh = l2 % H
            src = ((hh % 8) * 16 + 4 * t + l2 // H + 4 * (hh // 8)) & (LANES - 1)
            wqkv_ref[j * NT + t] = jnp.take_along_axis(c, src, axis=1)

    def permute_rows():
        for t in range(NT):
            for h in range(H):
                tmp_ref[t, h * WO_PITCH:h * WO_PITCH + Dh, :] = (
                    wo_in[h * Dh:(h + 1) * Dh, t * LANES:(t + 1) * LANES].astype(f32))
        for d in range(Dh):
            for t in range(NT):
                wo_ref[t, d * H // 2:(d + 1) * H // 2, :] = pltpu.bitcast(
                    tmp_ref[t, pl.ds(d, H, stride=WO_PITCH), :].astype(bf16), jnp.uint32)

    Q, K, V = 0, 1, 2

    def proj(xn, j, s, base=0, t0=0, nt=NT):
        r = jnp.dot(xn, _cat(wqkv_ref, j * NT + t0, nt), preferred_element_type=f32)
        for t in range(t0, t0 + nt):
            rt = r[:, (t - t0) * LANES:(t - t0 + 1) * LANES]
            if j == Q:
                qs[s][t, base:base + TS, :] = rt
            else:
                kvs[s][(j - 1) * NT + t, HALO + base:HALO + base + TS, :] = rt

    def qkv(xn, s):
        for j in (K, V, Q):
            proj(xn, j, s)

    def att(s, base=0, first=False, CH=8, NB=3):
        kv_ref = kvs[s]
        never = jnp.broadcast_to(never_ref[...], (CH, LANES)) > 0
        dens = {}
        pend = {}
        for c in range(TS // CH):
            o0 = c * CH
            r0 = base + o0
            sc = jnp.where(never, dens[c - NB], qscale) if c >= NB else qscale
            q = [qs[s][t, r0:r0 + CH, :] * sc for t in range(NT)]
            logits = []
            for w in range(W):
                s0 = HALO + r0 - DIL * w
                acc = q[0] * kv_ref[0, s0:s0 + CH, :]
                for t in range(1, NT):
                    acc = acc + q[t] * kv_ref[t, s0:s0 + CH, :]
                acc = acc + pltpu.roll(acc, 2 * H, 1)
                acc = acc + pltpu.roll(acc, H, 1)
                if first and o0 < DIL * w:
                    row = o0 + jax.lax.broadcasted_iota(jnp.int32, (CH, LANES), 0)
                    acc = jnp.where(row >= DIL * w, acc, -1e9 * LOG2E)
                logits.append(acc)
            m = logits[0]
            for w in range(1, W):
                m = jnp.maximum(m, logits[w])
            p = [jnp.exp2(lg - m) for lg in logits]
            den = p[0]
            for w in range(1, W):
                den = den + p[w]
            dens[c] = den
            inv = 1.0 / den
            for t in range(NT):
                acc = p[0] * kv_ref[NT + t, HALO + r0:HALO + r0 + CH, :]
                for w in range(1, W):
                    s0 = HALO + r0 - DIL * w
                    acc = acc + p[w] * kv_ref[NT + t, s0:s0 + CH, :]
                if c % 2 == 0:
                    pend[t] = acc * inv
                else:
                    both = jnp.concatenate([pend[t], acc * inv], axis=0)
                    atts[s][t, o0 - CH:o0 + CH, :] = both.astype(bf16)

    def halo(s, base=0):
        kvs[s][:, 0:HALO, :] = kvs[s][:, base + TS:base + TS + HALO, :]

    def halo_start(s, base):
        row0 = kvs[s][NT:, HALO + base:HALO + base + 1, :]
        kvs[s][NT:, base:base + HALO, :] = jnp.broadcast_to(row0, (NT, HALO, LANES))

    def oproj(s):
        return jnp.dot(_cat(atts[s], 0, NT), _cat(wo_ref, 0, NT), preferred_element_type=f32)

    def ln(x):
        return _layernorm(x).astype(bf16)

    def ll(x):
        return _layernorm(_layernorm(x)).astype(bf16)

    F = w1_ref.shape[0]
    FM = F // LANES * LANES
    nt_dims = (((1,), (1,)), ((), ()))

    def up(y, lo=0):
        hr = jax.lax.dot_general(w1_ref[FM:, :], y, nt_dims, preferred_element_type=f32).T
        h = jax.lax.dot_general(y, w1_ref[lo:FM, :], nt_dims, preferred_element_type=f32)
        h = jnp.concatenate([h, hr], axis=1)
        return _gelu_x2(h + b1_ref[...].astype(f32).reshape(1, -1)[:, lo:]).astype(bf16)

    def down(h, lo=0, n=NT):
        o = jnp.dot(h, w2_ref[:, lo * LANES:(lo + n) * LANES],
                    preferred_element_type=f32) * 0.5
        return o + b2_ref[...].astype(f32).reshape(1, -1)[:, lo * LANES:(lo + n) * LANES]

    def mlp(y):
        h1 = up(y, D)
        h0 = jax.lax.dot_general(y, w1_ref[:D, :], nt_dims, preferred_element_type=f32)
        h0 = _gelu_x2(h0 + b1_ref[...].astype(f32).reshape(1, -1)[:, :D]).astype(bf16)
        o = jnp.dot(h1, w2_ref[D:, :], preferred_element_type=f32)
        o = o + jnp.dot(h0, w2_ref[:D, :], preferred_element_type=f32)
        return o * 0.5 + b2_ref[...].astype(f32).reshape(1, -1)

    def put_y(v):
        for t in range(NT):
            y_ref[t] = v[:, t * LANES:(t + 1) * LANES]

    for g in range(NSEM):
        start(g)
    B0 = TS + HALO
    B1 = B0 + TS
    never_ref[...] = jnp.zeros((1, LANES), jnp.int32)
    kv0_ref[:NT, B0:B0 + HALO, :] = jnp.zeros((NT, HALO, LANES), f32)
    kv1_ref[:NT, 0:HALO, :] = jnp.zeros((NT, HALO, LANES), f32)

    wait(0)
    xn0 = ln(x_ref[0].astype(f32))
    wait(1)
    permute_cols(K)
    proj(xn0, K, 0, B0, 0, 2)
    wait(2)
    proj(xn0, K, 0, B0, 2, 2)
    xn1 = ln(x_ref[1].astype(f32))
    proj(xn1, K, 0, B1)
    xn2 = ln(x_ref[2].astype(f32))
    wait(3)
    proj(xn2, K, 0, 0, 0, 2)
    permute_cols(Q)
    proj(xn0, Q, 0, B0)
    wait(4)
    proj(xn2, K, 0, 0, 2, 2)
    permute_cols(V)
    permute_rows()
    proj(xn0, V, 0, B0)
    halo_start(0, B0)
    proj(xn1, V, 0, B1)
    halo(0, B1)
    proj(xn1, Q, 0, B1)
    att(0, B0, first=True, NB=5)
    xb_ref[...] = x_ref[0].astype(f32) + oproj(0)
    proj(xn2, Q, 0)
    y = ll(xb_ref[...])
    wait(5)
    m = mlp(y)
    att(0, B1)
    xb_ref[...] = xb_ref[...] + m
    xa_ref[...] = x_ref[1].astype(f32) + oproj(0)
    qkv(ln(xb_ref[...]), 1)
    halo_start(1, 0)
    m = mlp(ll(xa_ref[...]))
    att(1, first=True)
    halo(1)
    xa_ref[...] = xa_ref[...] + m
    xb_ref[...] = xb_ref[...] + oproj(1)
    proj(xn2, V, 0)
    put_y(ll(xb_ref[...]))
    wait(6)

    def body(j, carry):
        m = mlp(_cat(y_ref, 0, NT))
        att(0)
        halo(0)
        o_ref[j - 2] = (xb_ref[...] + m).astype(bf16)
        xn = ln(xa_ref[...])
        xb_ref[...] = xa_ref[...]
        xa_ref[...] = x_ref[j].astype(f32) + oproj(0)
        qkv(xn, 1)
        m = mlp(ll(xa_ref[...]))
        att(1)
        halo(1)
        xa_ref[...] = xa_ref[...] + m
        nxt = jnp.where(j + 1 < NBLK,
                        x_ref[jnp.minimum(j + 1, NBLK - 1)].astype(f32), xa_ref[...])
        xn = ln(nxt)
        xb_ref[...] = xb_ref[...] + oproj(1)
        qkv(xn, 0)
        put_y(ll(xb_ref[...]))
        o_copy(j - 2).start()
        return carry

    jax.lax.fori_loop(2, NBLK, body, 0)

    HD = D // 2
    kv0_ref[:, 0:HALO, :] = kv1_ref[:, 0:HALO, :]
    h = up(_cat(y_ref, 0, NT))
    att(0)
    o_ref[NBLK - 2, :, :HD] = (xb_ref[:, :HD] + down(h, 0, NT // 2)).astype(bf16)
    xa_ref[...] = xa_ref[...] + oproj(0)
    o_ref[NBLK - 2, :, HD:] = (xb_ref[:, HD:] + down(h, NT // 2, NT // 2)).astype(bf16)
    h = up(ll(xa_ref[...]))
    o_copy(NBLK - 2).start()
    for t in range(NT):
        cs = slice(t * LANES, (t + 1) * LANES)
        o_ref[NBLK - 1, :, cs] = (xa_ref[:, cs] + down(h, t, 1)).astype(bf16)
        o_last[t].start()
    for i in range(NBLK - 1):
        o_copy(i).wait()
    for c in o_last:
        c.wait()


@jax.jit
def pallas_interleave_layers__sliding_local_dilated__mixer_channel_mlp__prompt_kernel(
    A_x: jax.Array,
    A_wqkv: jax.Array,
    A_wo: jax.Array,
    B_x: jax.Array,
    B_w1: jax.Array,
    B_b1: jax.Array,
    B_w2: jax.Array,
    B_b2: jax.Array,
):
    B, S, D = A_x.shape
    F = B_w1.shape[1]
    assert B == 1 and D == 4 * LANES and S % TS == 0 and S // TS >= 4
    assert F % LANES != 0 and F % 16 == 0 and F > D + LANES
    NT = D // LANES
    NBLK = S // TS
    f32 = jnp.float32
    bf16 = jnp.bfloat16

    hbm = pl.BlockSpec(memory_space=pl.ANY)
    out = pl.pallas_call(
        functools.partial(_kernel, D=D, NBLK=NBLK),
        in_specs=[hbm] * 7,
        out_specs=hbm,
        out_shape=jax.ShapeDtypeStruct((S, D), A_x.dtype),
        scratch_shapes=[
            pltpu.VMEM((2 * NT, 3 * TS + 2 * HALO + 8, LANES), f32),
            pltpu.VMEM((2 * NT, TS + HALO, LANES), f32),
            pltpu.VMEM((NT, 3 * TS + HALO, LANES), f32),
            pltpu.VMEM((NT, TS, LANES), f32),
            pltpu.VMEM((NT, TS, LANES), bf16),
            pltpu.VMEM((NT, TS, LANES), bf16),
            pltpu.VMEM((TS, D), f32),
            pltpu.VMEM((TS, D), f32),
            pltpu.VMEM((NT, TS, LANES), bf16),
            pltpu.VMEM((3 * NT, D // 2, LANES), jnp.uint32),
            pltpu.VMEM((NT, D // 2, LANES), jnp.uint32),
            pltpu.VMEM((NT, H * WO_PITCH + 16, LANES), f32),
            pltpu.VMEM((NBLK, TS, D), bf16),
            pltpu.VMEM((NBLK, TS, D), bf16),
            pltpu.VMEM((3, D, D), bf16),
            pltpu.VMEM((D, D), bf16),
            pltpu.VMEM((F, D), bf16),
            pltpu.VMEM((F, D), bf16),
            pltpu.VMEM((F,), bf16),
            pltpu.VMEM((D,), bf16),
            pltpu.VMEM((1, LANES), jnp.int32),
            pltpu.SemaphoreType.DMA((NSEM,)),
        ],
        compiler_params=pltpu.CompilerParams(
            vmem_limit_bytes=100 * 1024 * 1024,
        ),
    )(A_x.reshape(NBLK, TS, D), A_wqkv, A_wo, B_w1.T, B_b1, B_w2, B_b2)
    return out.reshape(B, S, D)
```
